```python
import jax
import jax.numpy as jnp

def _softmax(x, axis=-1):
    return jax.nn.softmax(x, axis=axis)

def _gelu(x):
    return jax.nn.gelu(x, approximate=True)

def _silu(x):
    return jax.nn.silu(x)

def _sigmoid(x):
    return jax.nn.sigmoid(x)

def _layernorm(x, axis=-1, eps=1e-05):
    m = jnp.mean(x, axis=axis, keepdims=True)
    v = jnp.var(x, axis=axis, keepdims=True)
    return (x - m) / jnp.sqrt(v + eps)

def _scatter_add(tgt, idx, src, axis=0):
    return tgt.at[idx].add(src)

def _segment_sum(src, seg, n):
    return jax.ops.segment_sum(src, seg, n)

class _Rng:

    def __init__(self, key):
        self._k = key

    def _next(self):
        self._k, sub = jax.random.split(self._k)
        return sub

    def normal(self, shape):
        return jax.random.normal(self._next(), shape, dtype=jnp.bfloat16)

    def randint(self, lo, hi, shape):
        return jax.random.randint(self._next(), shape, lo, hi, dtype=jnp.int32)

    def uniform(self, shape, lo=0.0, hi=1.0):
        return jax.random.uniform(self._next(), shape, jnp.bfloat16, lo, hi)

    def permutation(self, n):
        return jax.random.permutation(self._next(), n)
kernel_name = 'gated_mix__ssm_conv_h3__memory_aug_recurrent_mem_tr__prompt'

def setup_inputs():
    _rng = _Rng(jax.random.key(int.from_bytes(__import__("os").urandom(4), "little")))
    _w = lambda a: (lambda t: t.astype(jnp.bfloat16) if jnp.issubdtype(t.dtype, jnp.floating) else t)(jnp.asarray(a))

    def _A_setup():
        B, S, D = (1, 2048, 1024)
        ks = 4
        return {'q': _w((lambda *s: _rng.normal(s) * 0.05)(B, S, D)), 'k': _w((lambda *s: _rng.normal(s) * 0.05)(B, S, D)), 'v': _w((lambda *s: _rng.normal(s) * 0.05)(B, S, D)), 'shift_k': _w((lambda *s: _rng.normal(s) * 0.05)(D, ks) * 0.5), 'ssm_k': _w((lambda *s: _rng.normal(s) * 0.05)(D, S) * (1.0 / S ** 0.5)), 'ssm_D': _w((lambda *s: _rng.normal(s) * 0.05)(D))}
    _A_in = _A_setup()

    def _B_setup():
        B, S, Dm = (1, 2048, 1024)
        H, Dh = (32, 128)
        M, seg = (8, 32)
        seg = min(seg, S)
        S = S // seg * seg
        return {'x': _w((lambda *s: _rng.normal(s) * 0.05)(B, S, Dm)), 'mem0': _w((lambda *s: _rng.normal(s) * 0.05)(B, M, Dm)), 'Wq': _w((lambda *s: _rng.normal(s) * 0.05)(Dm, H, Dh) * Dm ** (-0.5)), 'Wk': _w((lambda *s: _rng.normal(s) * 0.05)(Dm, H, Dh) * Dm ** (-0.5)), 'Wv': _w((lambda *s: _rng.normal(s) * 0.05)(Dm, H, Dh) * Dm ** (-0.5)), 'Wo': _w((lambda *s: _rng.normal(s) * 0.05)(H, Dh, Dm) * (H * Dh) ** (-0.5)), 'seg_len': seg}
    _B_in = _B_setup()
    return {'A_q': _A_in['q'], 'A_k': _A_in['k'], 'A_v': _A_in['v'], 'A_shift_k': _A_in['shift_k'], 'A_ssm_k': _A_in['ssm_k'], 'A_ssm_D': _A_in['ssm_D'], 'B_x': _B_in['x'], 'B_mem0': _B_in['mem0'], 'B_Wq': _B_in['Wq'], 'B_Wk': _B_in['Wk'], 'B_Wv': _B_in['Wv'], 'B_Wo': _B_in['Wo'], 'B_seg_len': _B_in['seg_len'], 'gate_w': _w((lambda *s: _rng.normal(s) * 0.05)(1024))}

def reference(A_q, A_k, A_v, A_shift_k, A_ssm_k, A_ssm_D, B_x, B_mem0, B_Wq, B_Wk, B_Wv, B_Wo, B_seg_len, gate_w):

    def _A_ref(q, k, v, shift_k, ssm_k, ssm_D):
        B, S, D = q.shape
        ks = shift_k.shape[-1]
        k_pad = jnp.pad(k, ((0, 0), (ks - 1, 0), (0, 0)))
        k_shift = jnp.zeros_like(k)
        for t in range(ks):
            k_shift = k_shift + k_pad[:, t:t + S, :] * shift_k[:, ks - 1 - t][None, None, :]
        kv = k_shift * v
        L = 2 * S
        kv_pad = jnp.pad(kv, ((0, 0), (0, S), (0, 0)))
        kf_pad = jnp.pad(ssm_k, ((0, 0), (0, S)))
        kv_f = (lambda x, axes=(-2, -1): jnp.fft.rfft2(x.astype(jnp.float32), axes=axes))(kv_pad[:, None, :, :], axes=(1, 2))
        kf_f = (lambda x, axes=(-2, -1): jnp.fft.rfft2(x.astype(jnp.float32), axes=axes))(kf_pad[:, None, :], axes=(1, 2))
        kf_f = (lambda x, *d: x.transpose(*d))(kf_f, 1, 2, 0)
        y_f = kv_f * kf_f[None, :, :, :]
        y = (lambda x, s, axes=(-2, -1): jnp.fft.irfft2(x, s=s, axes=axes).astype(jnp.bfloat16))(y_f, (1, L), axes=(1, 2))[:, 0, :S, :]
        y = y + kv * ssm_D[None, None, :]
        return q * y

    def _B_ref(x, mem0, Wq, Wk, Wv, Wo, seg_len):
        B, S, Dm = x.shape
        H, Dh = (Wq.shape[1], Wq.shape[2])
        M = mem0.shape[1]
        scale = Dh ** (-0.5)
        n_seg = S // seg_len
        L = M + seg_len
        idx = jnp.arange(L)
        mask = (idx[:, None] < M) | (idx[:, None] >= idx[None, :])
        mem = mem0
        outs = []
        for s in range(n_seg):
            xs = x[:, s * seg_len:(s + 1) * seg_len, :].copy()
            h = jnp.concatenate([mem, xs], axis=1)
            q = jnp.einsum('btd,dhe->bhte', h, Wq)
            k = jnp.einsum('btd,dhe->bhte', h, Wk)
            v = jnp.einsum('btd,dhe->bhte', h, Wv)
            scores = jnp.einsum('bhqe,bhke->bhqk', q, k) * scale
            scores = jnp.where(mask[None, None], scores, -1000000000.0)
            p = _softmax(scores, axis=-1)
            o = jnp.einsum('bhqk,bhke->bhqe', p, v)
            o = jnp.einsum('bhte,hed->btd', o, Wo)
            mem = o[:, :M, :].copy()
            outs.append(o[:, M:, :])
        return jnp.concatenate(outs, axis=1)
    x = A_q
    g = _sigmoid((x * gate_w).sum(-1, keepdims=True))
    a = _A_ref(x, A_k, A_v, A_shift_k, A_ssm_k, A_ssm_D)
    b = _B_ref(x, B_mem0, B_Wq, B_Wk, B_Wv, B_Wo, B_seg_len)
    return g * a + (1 - g) * b
```

```python
import functools

import jax
import jax.numpy as jnp
import numpy as np
from jax.experimental import pallas as pl
from jax.experimental.pallas import tpu as pltpu

S, D = 2048, 1024
H, DH = 32, 128
M, SEG = 8, 32
NSEG = S // SEG
KS = 4
CT = 256
NCT = D // CT
GH = 4
NG = H // GH
GW = GH * DH
ROWS = 48
NFFT = 2 * S


def _fft_constants():
    n1 = np.arange(16)
    k1 = np.arange(16)
    c = np.exp(-1j * np.pi * np.outer(2 * k1 + 1, n1) / 32.0)
    gf = np.concatenate([c.real, c.imag], axis=0)
    gi = np.concatenate([c.real.T, c.imag.T], axis=1) * (2.0 / NFFT)
    eye = np.eye(8)
    gf8 = np.kron(gf, eye)
    gi8 = np.kron(gi, eye)
    n2 = np.arange(128)
    k2 = np.arange(128)
    f = np.zeros((16, 256, 256))
    for a in range(16):
        m = np.exp(-2j * np.pi * np.outer(a + 0.5 + 32.0 * k2, n2) / NFFT)
        f[a] = np.block([[m.real, -m.imag], [m.imag, m.real]])
    ft = np.transpose(f, (0, 2, 1))
    return (gf8.astype(np.float32), gi8.astype(np.float32),
            f.astype(np.float32), ft.astype(np.float32))


_GF8, _GI8, _F, _FT = _fft_constants()


def _kernel(p_ref, mem0_ref, gf_ref, gi_ref,
            q_hbm, k_hbm, v_hbm, h_hbm, wq_hbm, wk_hbm, wv_hbm, wo_hbm, f_hbm, ft_hbm,
            out_hbm,
            x_s, o_s, g_s, wqkv_s, wo_s, st_s, kin_s, vin_s, hin_s,
            kpad_s, kv_s, hf_s, a_s, ah_s, f_s, ft_s,
            sem_in, sem_st, sem_misc, sem_wo, sem_out):
    bf16, f32 = jnp.bfloat16, jnp.float32

    def tile_copies(i, slot):
        c0 = pl.multiple_of(i * CT, CT)
        return (
            pltpu.make_async_copy(k_hbm.at[:, pl.ds(c0, CT)], kin_s.at[slot], sem_in.at[0, slot]),
            pltpu.make_async_copy(v_hbm.at[:, pl.ds(c0, CT)], vin_s.at[slot], sem_in.at[1, slot]),
            pltpu.make_async_copy(h_hbm.at[pl.ds(c0, CT), :], hin_s.at[slot], sem_in.at[2, slot]),
        )

    misc = (
        pltpu.make_async_copy(f_hbm, f_s, sem_misc.at[0]),
        pltpu.make_async_copy(ft_hbm, ft_s, sem_misc.at[1]),
        pltpu.make_async_copy(q_hbm, x_s, sem_misc.at[2]),
    )
    w_srcs = (wq_hbm, wk_hbm, wv_hbm)

    def st_copy(m):
        return pltpu.make_async_copy(w_srcs[m], st_s.at[m % 2], sem_st.at[m % 2])

    def wo_copy(j):
        return pltpu.make_async_copy(wo_hbm.at[:, pl.ds(j * 128, 128)], wo_s.at[j], sem_wo.at[j])

    for c in tile_copies(0, 0):
        c.start()
    for c in misc:
        c.start()
    for c in tile_copies(1, 1):
        c.start()
    st_copy(0).start()
    st_copy(1).start()

    gf = gf_ref[...]
    gi = gi_ref[...]
    kpad_s[0:8, :] = jnp.zeros((8, CT), f32)

    misc[2].wait()
    gate_w = p_ref[5:6, :]

    def gate_body(r, carry):
        r0 = pl.multiple_of(r * 128, 128)
        xf = x_s[pl.ds(r0, 128), :].astype(f32) * gate_w
        sm = jnp.sum(xf, axis=-1, keepdims=True)
        g = 1.0 / (1.0 + jnp.exp(-sm))
        g_s[pl.ds(r0, 128), :] = jnp.broadcast_to(g, (128, 128))
        return carry

    jax.lax.fori_loop(0, S // 128, gate_body, 0)

    def branch_a(i, slot):
        c0 = pl.multiple_of(i * CT, CT)
        for c in tile_copies(i, slot):
            c.wait()

        def cvt_body(r, carry):
            r0 = pl.multiple_of(r * 256, 256)
            kpad_s[pl.ds(8 + r0, 256), :] = kin_s[slot, pl.ds(r0, 256), :].astype(f32)
            kv_s[pl.ds(r0, 256), :] = vin_s[slot, pl.ds(r0, 256), :].astype(f32)
            return carry

        jax.lax.fori_loop(0, S // 256, cvt_body, 0)
        hf_s[...] = hin_s[slot].astype(f32)

        pt = p_ref[:, pl.ds(c0, CT)]
        taps = [pt[j:j + 1, :] for j in range(KS)]
        dvec = pt[4:5, :]

        def s1_body(j, carry):
            j8 = pl.multiple_of(j * 8, 8)
            blocks = []
            for n1 in range(16):
                r0 = pl.multiple_of(n1 * 128 + j8, 8)
                win = kpad_s[pl.ds(r0, 16), :]
                acc = win[8:16] * taps[0]
                for t in range(1, KS):
                    acc = acc + win[8 - t:16 - t] * taps[t]
                kv = acc * kv_s[pl.ds(r0, 8), :]
                kv_s[pl.ds(r0, 8), :] = kv
                blocks.append(kv)
            rhs = jnp.concatenate(blocks, axis=0).astype(bf16)
            out = jnp.dot(gf, rhs, preferred_element_type=f32)
            for ks in range(32):
                a_s[ks, pl.ds(j8, 8), :] = out[ks * 8:(ks + 1) * 8, :]
            return carry

        jax.lax.fori_loop(0, 16, s1_body, 0, unroll=2)

        def h1_body(j, carry):
            j8 = pl.multiple_of(j * 16, 16)
            lo = hf_s[pl.ds(j8, 8), :]
            hi = hf_s[pl.ds(j8 + 8, 8), :]
            blocks = [jnp.concatenate([lo[:, n1 * 128:(n1 + 1) * 128],
                                       hi[:, n1 * 128:(n1 + 1) * 128]], axis=1)
                      for n1 in range(16)]
            rhs = jnp.concatenate(blocks, axis=0).astype(bf16)
            out = jnp.dot(gf, rhs, preferred_element_type=f32)
            for ks in range(32):
                ah_s[ks, pl.ds(j8, 8), :] = out[ks * 8:(ks + 1) * 8, 0:128]
                ah_s[ks, pl.ds(j8 + 8, 8), :] = out[ks * 8:(ks + 1) * 8, 128:256]
            return carry

        jax.lax.fori_loop(0, CT // 16, h1_body, 0, unroll=2)

        def s2_body(k1, carry):
            fk = f_s[k1]
            a = jnp.concatenate([a_s[k1], a_s[16 + k1]], axis=0).astype(bf16)
            xs = jnp.dot(fk, a, preferred_element_type=f32)
            ah = jnp.concatenate([ah_s[k1], ah_s[16 + k1]], axis=1).astype(bf16)
            hs = jax.lax.dot_general(fk, ah, (((1,), (1,)), ((), ())),
                                     preferred_element_type=f32)
            xr, xi = xs[0:128], xs[128:256]
            hr, hi = hs[0:128], hs[128:256]
            y = jnp.concatenate([xr * hr - xi * hi, xr * hi + xi * hr], axis=0).astype(bf16)
            b = jnp.dot(ft_s[k1], y, preferred_element_type=f32)
            a_s[k1] = b[0:128]
            a_s[16 + k1] = b[128:256]
            return carry

        jax.lax.fori_loop(0, 16, s2_body, 0, unroll=2)

        def inv_body(jj, carry):
            j16 = pl.multiple_of(jj * 16, 16)
            ys = []
            for u in range(2):
                rhs = jnp.concatenate(
                    [a_s[ks, pl.ds(j16 + 8 * u, 8), :] for ks in range(32)], axis=0).astype(bf16)
                ys.append(jnp.dot(gi, rhs, preferred_element_type=f32))
            for n1 in range(16):
                r0 = pl.multiple_of(n1 * 128 + j16, 16)
                y = jnp.concatenate([ys[0][n1 * 8:(n1 + 1) * 8], ys[1][n1 * 8:(n1 + 1) * 8]], axis=0)
                y = y + kv_s[pl.ds(r0, 16), :] * dvec
                qv = x_s[pl.ds(r0, 16), pl.ds(c0, CT)].astype(f32)
                g = g_s[pl.ds(r0, 16), :]
                g = jnp.concatenate([g] * (CT // 128), axis=1)
                o_s[pl.ds(r0, 16), pl.ds(c0, CT)] = (g * (qv * y)).astype(bf16)
            return carry

        jax.lax.fori_loop(0, 8, inv_body, 0)

    def repack(m):
        s32 = st_s.at[m % 2].bitcast(jnp.uint32)

        def body(c, carry):
            r0 = pl.multiple_of(c * 64, 64)
            for hp in range(H // 2):
                w = s32[c, pl.ds(hp, 128, stride=16), :]
                lo = pltpu.bitcast(w << 16, f32).astype(bf16)
                hi = pltpu.bitcast(w & jnp.uint32(0xFFFF0000), f32).astype(bf16)
                for hh, val in ((2 * hp, lo), (2 * hp + 1, hi)):
                    g, e = hh // GH, hh % GH
                    wqkv_s[m, g, pl.ds(r0, 64), e * 128:(e + 1) * 128] = pltpu.bitcast(val, jnp.uint32)
            return carry

        jax.lax.fori_loop(0, D // 128, body, 0)

    misc[0].wait()
    misc[1].wait()

    def phase1(i, carry):
        slot = i % 2
        branch_a(i, slot)

        @pl.when(i + 2 < NCT)
        def _():
            for c in tile_copies(i + 2, slot):
                c.start()

        @pl.when(i == 0)
        def _():
            st_copy(0).wait()
            repack(0)
            st_copy(2).start()

        @pl.when(i == 1)
        def _():
            st_copy(1).wait()
            repack(1)
            for j in range(D // 128):
                wo_copy(j).start()

        @pl.when(i == 2)
        def _():
            st_copy(2).wait()
            repack(2)

        return carry

    jax.lax.fori_loop(0, NCT, phase1, 0)
    for j in range(D // 128):
        wo_copy(j).wait()

    row = jax.lax.broadcasted_iota(jnp.int32, (ROWS, ROWS), 0)
    col = jax.lax.broadcasted_iota(jnp.int32, (ROWS, ROWS), 1)
    valid = (col < M) | (col >= 16)
    mask = valid & ((row < 16) | (col <= row))
    scale = DH ** -0.5

    def getw(m, g):
        return pltpu.bitcast(wqkv_s[m, g], bf16)

    def getwo(g):
        return jnp.concatenate([wo_s[j, g * GW:(g + 1) * GW, :] for j in range(D // 128)], axis=1)

    def qkv(hb, g):
        return tuple(jnp.dot(hb, getw(m, g), preferred_element_type=f32).astype(bf16)
                     for m in range(3))

    def attn(t):
        q, k, v = t
        outs = []
        for e in range(GH):
            sl = slice(e * 128, (e + 1) * 128)
            s = jax.lax.dot_general(q[:, sl], k[:, sl], (((1,), (1,)), ((), ())),
                                    preferred_element_type=f32)
            s = jnp.where(mask, s * scale, -1e9)
            mx = jnp.max(s, axis=-1, keepdims=True)
            ex = jnp.exp(s - mx)
            sm = jnp.sum(ex, axis=-1, keepdims=True)
            p = (ex / sm).astype(bf16)
            outs.append(jnp.dot(p, v[:, sl], preferred_element_type=f32).astype(bf16))
        return jnp.concatenate(outs, axis=1)

    def out_copy(s):
        r0 = pl.multiple_of(s * SEG, SEG)
        return pltpu.make_async_copy(o_s.at[pl.ds(r0, SEG), :], out_hbm.at[pl.ds(r0, SEG), :], sem_out)

    LAG = 3

    def step(s, mem):
        r0 = pl.multiple_of(s * SEG, SEG)
        top = jnp.concatenate([mem, jnp.zeros((8, D), f32)], axis=0).astype(bf16)
        hb = jnp.concatenate([top, x_s[pl.ds(r0, SEG), :]], axis=0)
        ts, os_ = {}, {}
        acc = None
        for g in range(NG + LAG):
            if g < NG:
                ts[g] = qkv(hb, g)
            if 1 <= g <= NG:
                os_[g - 1] = attn(ts[g - 1])
            if g >= LAG:
                d = jnp.dot(os_[g - LAG], getwo(g - LAG), preferred_element_type=f32)
                acc = d if acc is None else acc + d
        gb = g_s[pl.ds(r0, SEG), :]
        gb = jnp.concatenate([gb] * (D // 128), axis=1)
        res = o_s[pl.ds(r0, SEG), :].astype(f32) + (1.0 - gb) * acc[16:48]
        o_s[pl.ds(r0, SEG), :] = res.astype(bf16)
        out_copy(s).start()
        return acc[0:8]

    jax.lax.fori_loop(0, NSEG, step, mem0_ref[...].astype(f32))
    pltpu.make_async_copy(o_s, out_hbm, sem_out).wait()


@functools.partial(jax.jit, static_argnames=("B_seg_len",))
def pallas_gated_mix__ssm_conv_h3__memory_aug_recurrent_mem_tr__prompt_kernel(
    A_q, A_k, A_v, A_shift_k, A_ssm_k, A_ssm_D, B_x, B_mem0,
    B_Wq, B_Wk, B_Wv, B_Wo, B_seg_len, gate_w,
):
    assert B_seg_len == SEG
    f32, bf16 = jnp.float32, jnp.bfloat16
    params = jnp.concatenate(
        [A_shift_k.T.astype(f32), A_ssm_D.reshape(1, D).astype(f32),
         gate_w.reshape(1, D).astype(f32), jnp.zeros((2, D), f32)], axis=0)
    hbm = pl.BlockSpec(memory_space=pl.ANY)
    vmem = pl.BlockSpec(memory_space=pltpu.VMEM)
    out = pl.pallas_call(
        _kernel,
        out_shape=jax.ShapeDtypeStruct((S, D), bf16),
        in_specs=[vmem, vmem, vmem, vmem] + [hbm] * 10,
        out_specs=hbm,
        scratch_shapes=[
            pltpu.VMEM((S, D), bf16),
            pltpu.VMEM((S, D), bf16),
            pltpu.VMEM((S, 128), f32),
            pltpu.VMEM((3, NG, D // 2, GW), jnp.uint32),
            pltpu.VMEM((D // 128, H * DH, 128), bf16),
            pltpu.VMEM((2, D // 128, 128 * H, DH), bf16),
            pltpu.VMEM((2, S, CT), bf16),
            pltpu.VMEM((2, S, CT), bf16),
            pltpu.VMEM((2, CT, S), bf16),
            pltpu.VMEM((8 + S, CT), f32),
            pltpu.VMEM((S, CT), f32),
            pltpu.VMEM((CT, S), f32),
            pltpu.VMEM((32, 128, CT), f32),
            pltpu.VMEM((32, CT, 128), f32),
            pltpu.VMEM((16, 256, 256), bf16),
            pltpu.VMEM((16, 256, 256), bf16),
            pltpu.SemaphoreType.DMA((3, 2)),
            pltpu.SemaphoreType.DMA((2,)),
            pltpu.SemaphoreType.DMA((3,)),
            pltpu.SemaphoreType.DMA((D // 128,)),
            pltpu.SemaphoreType.DMA(()),
        ],
        compiler_params=pltpu.CompilerParams(vmem_limit_bytes=112 * 1024 * 1024),
    )(
        params, B_mem0.reshape(M, D), jnp.asarray(_GF8, bf16), jnp.asarray(_GI8, bf16),
        A_q.reshape(S, D), A_k.reshape(S, D), A_v.reshape(S, D), A_ssm_k,
        B_Wq.reshape(D // 128, 128 * H, DH), B_Wk.reshape(D // 128, 128 * H, DH), B_Wv.reshape(D // 128, 128 * H, DH),
        B_Wo.reshape(H * DH, D), jnp.asarray(_F, bf16), jnp.asarray(_FT, bf16),
    )
    return out.reshape(1, S, D)
```

```python
import functools

import jax
import jax.numpy as jnp
import numpy as np
from jax.experimental import pallas as pl
from jax.experimental.pallas import tpu as pltpu

S, D = 2048, 1024
H, DH = 32, 128
M, SEG = 8, 32
NSEG = S // SEG
KS = 4
CT = 256
NCT = D // CT
GH = 4
NG = H // GH
GW = GH * DH
ROWS = 48
NFFT = 2 * S
LAG = 3


def _fft_constants():
    n1 = np.arange(16)
    k1 = np.arange(16)
    c = np.exp(-1j * np.pi * np.outer(2 * k1 + 1, n1) / 32.0)
    gf = np.concatenate([c.real, c.imag], axis=0)
    gi = np.concatenate([c.real.T, c.imag.T], axis=1) * (2.0 / NFFT)
    eye = np.eye(8)
    gf8 = np.kron(gf, eye)
    gi8 = np.kron(gi, eye)
    n2 = np.arange(128)
    k2 = np.arange(128)
    f = np.zeros((16, 256, 256))
    for a in range(16):
        m = np.exp(-2j * np.pi * np.outer(a + 0.5 + 32.0 * k2, n2) / NFFT)
        f[a] = np.block([[m.real, -m.imag], [m.imag, m.real]])
    ft = np.transpose(f, (0, 2, 1))
    return (gf8.astype(np.float32), gi8.astype(np.float32),
            f.astype(np.float32), ft.astype(np.float32))


_GF8, _GI8, _F, _FT = _fft_constants()


def _kernel(p_ref, mem0_ref, gf_ref, gi_ref,
            q_hbm, k_hbm, v_hbm, h_hbm, wq_hbm, wk_hbm, wv_hbm, wo_hbm, f_hbm, ft_hbm,
            out_hbm,
            x_s, o_s, g_s, wqkv_s, wo_s, st_s, kin_s, vin_s, hin_s,
            kpad_s, kv_s, hf_s, a_s, ah_s, f_s, ft_s, stash_s,
            sem_in, sem_st, sem_misc, sem_wo, sem_out):
    bf16, f32 = jnp.bfloat16, jnp.float32

    def tile_copies(i, slot):
        c0 = pl.multiple_of(i * CT, CT)
        return (
            pltpu.make_async_copy(k_hbm.at[:, pl.ds(c0, CT)], kin_s.at[slot], sem_in.at[0, slot]),
            pltpu.make_async_copy(v_hbm.at[:, pl.ds(c0, CT)], vin_s.at[slot], sem_in.at[1, slot]),
            pltpu.make_async_copy(h_hbm.at[pl.ds(c0, CT), :], hin_s.at[slot], sem_in.at[2, slot]),
        )

    misc = (
        pltpu.make_async_copy(f_hbm, f_s, sem_misc.at[0]),
        pltpu.make_async_copy(ft_hbm, ft_s, sem_misc.at[1]),
        pltpu.make_async_copy(q_hbm, x_s, sem_misc.at[2]),
    )
    w_srcs = (wq_hbm, wk_hbm, wv_hbm)

    def st_copy(m):
        return pltpu.make_async_copy(w_srcs[m], st_s.at[m], sem_st.at[m])

    def wo_copy(j):
        return pltpu.make_async_copy(wo_hbm.at[:, pl.ds(j * 128, 128)], wo_s.at[j], sem_wo.at[j])

    for c in tile_copies(0, 0):
        c.start()
    for c in misc[:2]:
        c.start()

    gf = gf_ref[...]
    gi = gi_ref[...]
    kpad_s[0:8, :] = jnp.zeros((8, CT), f32)

    gate_w = p_ref[5:6, :]

    def gate_body(r, carry):
        r0 = pl.multiple_of(r * 128, 128)
        xf = x_s[pl.ds(r0, 128), :].astype(f32) * gate_w
        sm = jnp.sum(xf, axis=-1, keepdims=True)
        g = 1.0 / (1.0 + jnp.exp(-sm))
        g_s[pl.ds(r0, 128), :] = jnp.broadcast_to(g, (128, 128))
        return carry


    def branch_a(i, slot):
        c0 = pl.multiple_of(i * CT, CT)
        for c in tile_copies(i, slot):
            c.wait()

        def cvt_body(r, carry):
            r0 = pl.multiple_of(r * 256, 256)
            kpad_s[pl.ds(8 + r0, 256), :] = kin_s[slot, pl.ds(r0, 256), :].astype(f32)
            kv_s[pl.ds(r0, 256), :] = vin_s[slot, pl.ds(r0, 256), :].astype(f32)
            return carry

        jax.lax.fori_loop(0, S // 256, cvt_body, 0)

        @pl.when(i == 0)
        def _():
            misc[2].start()
            for c in tile_copies(1, 1):
                c.start()

        hf_s[...] = hin_s[slot].astype(f32)

        pt = p_ref[:, pl.ds(c0, CT)]
        taps = [pt[j:j + 1, :] for j in range(KS)]
        dvec = pt[4:5, :]

        def s1_body(j, carry):
            j8 = pl.multiple_of(j * 8, 8)
            blocks = []
            for n1 in range(16):
                r0 = pl.multiple_of(n1 * 128 + j8, 8)
                win = kpad_s[pl.ds(r0, 16), :]
                acc = win[8:16] * taps[0]
                for t in range(1, KS):
                    acc = acc + win[8 - t:16 - t] * taps[t]
                kv = acc * kv_s[pl.ds(r0, 8), :]
                kv_s[pl.ds(r0, 8), :] = kv
                blocks.append(kv)
            rhs = jnp.concatenate(blocks, axis=0).astype(bf16)
            out = jnp.dot(gf, rhs, preferred_element_type=f32)
            for ks in range(32):
                a_s[ks, pl.ds(j8, 8), :] = out[ks * 8:(ks + 1) * 8, :]
            return carry

        jax.lax.fori_loop(0, 16, s1_body, 0, unroll=2)

        @pl.when(i == 0)
        def _():
            st_copy(0).start()
            misc[0].wait()
            misc[1].wait()


        def h1_body(j, carry):
            j8 = pl.multiple_of(j * 16, 16)
            lo = hf_s[pl.ds(j8, 8), :]
            hi = hf_s[pl.ds(j8 + 8, 8), :]
            blocks = [jnp.concatenate([lo[:, n1 * 128:(n1 + 1) * 128],
                                       hi[:, n1 * 128:(n1 + 1) * 128]], axis=1)
                      for n1 in range(16)]
            rhs = jnp.concatenate(blocks, axis=0).astype(bf16)
            out = jnp.dot(gf, rhs, preferred_element_type=f32)
            for ks in range(32):
                ah_s[ks, pl.ds(j8, 8), :] = out[ks * 8:(ks + 1) * 8, 0:128]
                ah_s[ks, pl.ds(j8 + 8, 8), :] = out[ks * 8:(ks + 1) * 8, 128:256]
            return carry

        jax.lax.fori_loop(0, CT // 16, h1_body, 0, unroll=2)

        def s2_body(k1, carry):
            fk = f_s[k1]
            a = jnp.concatenate([a_s[k1], a_s[16 + k1]], axis=0).astype(bf16)
            xs = jnp.dot(fk, a, preferred_element_type=f32)
            ah = jnp.concatenate([ah_s[k1], ah_s[16 + k1]], axis=1).astype(bf16)
            hs = jax.lax.dot_general(fk, ah, (((1,), (1,)), ((), ())),
                                     preferred_element_type=f32)
            xr, xi = xs[0:128], xs[128:256]
            hr, hi = hs[0:128], hs[128:256]
            y = jnp.concatenate([xr * hr - xi * hi, xr * hi + xi * hr], axis=0).astype(bf16)
            b = jnp.dot(ft_s[k1], y, preferred_element_type=f32)
            a_s[k1] = b[0:128]
            a_s[16 + k1] = b[128:256]
            return carry

        jax.lax.fori_loop(0, 16, s2_body, 0, unroll=2)

        @pl.when(i == 0)
        def _():
            st_copy(1).start()
            misc[2].wait()
            jax.lax.fori_loop(0, S // 128, gate_body, 0)


        def inv_body(jj, carry):
            j16 = pl.multiple_of(jj * 16, 16)
            ys = []
            for u in range(2):
                rhs = jnp.concatenate(
                    [a_s[ks, pl.ds(j16 + 8 * u, 8), :] for ks in range(32)], axis=0).astype(bf16)
                ys.append(jnp.dot(gi, rhs, preferred_element_type=f32))
            for n1 in range(16):
                r0 = pl.multiple_of(n1 * 128 + j16, 16)
                y = jnp.concatenate([ys[0][n1 * 8:(n1 + 1) * 8], ys[1][n1 * 8:(n1 + 1) * 8]], axis=0)
                y = y + kv_s[pl.ds(r0, 16), :] * dvec
                qv = x_s[pl.ds(r0, 16), pl.ds(c0, CT)].astype(f32)
                g = g_s[pl.ds(r0, 16), :]
                g = jnp.concatenate([g] * (CT // 128), axis=1)
                o_s[pl.ds(r0, 16), pl.ds(c0, CT)] = (g * (qv * y)).astype(bf16)
            return carry

        jax.lax.fori_loop(0, 8, inv_body, 0)

    def repack(m):
        s32 = st_s.at[m].bitcast(jnp.uint32)

        def body(c, carry):
            r0 = pl.multiple_of(c * 64, 64)
            for hp in range(H // 2):
                w = s32[c, pl.ds(hp, 128, stride=16), :]
                lo = pltpu.bitcast(w << 16, f32).astype(bf16)
                hi = pltpu.bitcast(w & jnp.uint32(0xFFFF0000), f32).astype(bf16)
                for hh, val in ((2 * hp, lo), (2 * hp + 1, hi)):
                    g, e = hh // GH, hh % GH
                    wqkv_s[m, g, pl.ds(r0, 64), e * 128:(e + 1) * 128] = pltpu.bitcast(val, jnp.uint32)
            return carry

        jax.lax.fori_loop(0, D // 128, body, 0)

    def phase1(i, carry):
        slot = i % 2
        branch_a(i, slot)

        @pl.when(i + 2 < NCT)
        def _():
            for c in tile_copies(i + 2, slot):
                c.start()

        @pl.when(i == 0)
        def _():
            st_copy(2).start()

        @pl.when(i == 1)
        def _():
            for j in range(D // 128):
                wo_copy(j).start()

        for m in range(3):
            @pl.when(i == m + 1)
            def _():
                st_copy(m).wait()
                repack(m)

        return carry

    jax.lax.fori_loop(0, NCT, phase1, 0)
    for j in range(D // 128):
        wo_copy(j).wait()

    row = jax.lax.broadcasted_iota(jnp.int32, (ROWS, ROWS), 0)
    col = jax.lax.broadcasted_iota(jnp.int32, (ROWS, ROWS), 1)
    mask0 = ((col < M) | (col >= 16)) & ((row < 16) | (col <= row))
    mask1 = ((col < 16) | (col >= 24)) & ((row < M) | (col <= row))
    scale = DH ** -0.5

    def getw(m, g):
        return pltpu.bitcast(wqkv_s[m, g], bf16)

    def getwo(g):
        return jnp.concatenate([wo_s[j, g * GW:(g + 1) * GW, :] for j in range(D // 128)], axis=1)

    def attn(q, k, v, mask):
        outs = []
        for e in range(GH):
            sl = slice(e * 128, (e + 1) * 128)
            s = jax.lax.dot_general(q[:, sl], k[:, sl], (((1,), (1,)), ((), ())),
                                    preferred_element_type=f32)
            s = jnp.where(mask, s * scale, -1e9)
            mx = jnp.max(s, axis=-1, keepdims=True)
            ex = jnp.exp(s - mx)
            sm = jnp.sum(ex, axis=-1, keepdims=True)
            p = (ex / sm).astype(bf16)
            outs.append(jnp.dot(p, v[:, sl], preferred_element_type=f32))
        return jnp.concatenate(outs, axis=1)

    def out_copy(j):
        r0 = pl.multiple_of(j * 2 * SEG, 2 * SEG)
        return pltpu.make_async_copy(o_s.at[pl.ds(r0, 2 * SEG), :],
                                     out_hbm.at[pl.ds(r0, 2 * SEG), :], sem_out)

    def half_step(hb, even):
        ts, os_ = {}, {}
        acc = None
        for g in range(NG + LAG):
            cs = slice(g * GW, (g + 1) * GW)
            if g < NG:
                ts[g] = tuple(jnp.dot(hb, getw(m, g), preferred_element_type=f32) for m in range(3))
            if 1 <= g <= NG:
                a = g - 1
                ca = slice(a * GW, (a + 1) * GW)
                if even:
                    for m in range(3):
                        stash_s[m, :, ca] = ts[a][m][8:16]
                    q, k, v = (t.astype(bf16) for t in ts[a])
                    o = attn(q, k, v, mask0)
                    stash_s[3, :, ca] = o[40:48]
                    os_[a] = jnp.concatenate([o[0:8], o[16:40]], axis=0).astype(bf16)
                else:
                    q, k, v = (jnp.concatenate(
                        [jnp.concatenate([ts[a][m][0:8], stash_s[m, :, ca]], axis=0).astype(bf16),
                         ts[a][m].astype(bf16)], axis=0) for m in range(3))
                    o = attn(q, k, v, mask1)
                    os_[a] = jnp.concatenate([o[0:16], stash_s[3, :, ca], o[24:48]], axis=0).astype(bf16)
            if g >= LAG:
                d = jnp.dot(os_[g - LAG], getwo(g - LAG), preferred_element_type=f32)
                acc = d if acc is None else acc + d
        return acc

    def step(j, mem):
        r0 = pl.multiple_of(j * 2 * SEG, 2 * SEG)
        xa = x_s[pl.ds(r0, SEG), :]
        xb = x_s[pl.ds(r0 + SEG, 16), :].astype(f32)
        xc = x_s[pl.ds(r0 + SEG + 16, 16), :]
        hb = jnp.concatenate([jnp.concatenate([mem, xb[0:8]], axis=0).astype(bf16), xa], axis=0)
        acc0 = half_step(hb, True)
        hb = jnp.concatenate([jnp.concatenate([acc0[0:8], xb[8:16]], axis=0).astype(bf16), xc], axis=0)
        acc1 = half_step(hb, False)
        b = jnp.concatenate([acc0[8:32], acc1[16:24], acc1[8:16], acc1[24:48]], axis=0)
        gb = g_s[pl.ds(r0, 2 * SEG), :]
        gb = jnp.concatenate([gb] * (D // 128), axis=1)
        res = o_s[pl.ds(r0, 2 * SEG), :].astype(f32) + (1.0 - gb) * b
        o_s[pl.ds(r0, 2 * SEG), :] = res.astype(bf16)
        out_copy(j).start()
        return acc1[0:8]

    jax.lax.fori_loop(0, NSEG // 2, step, mem0_ref[...].astype(f32))
    pltpu.make_async_copy(o_s, out_hbm, sem_out).wait()


@functools.partial(jax.jit, static_argnames=("B_seg_len",))
def pallas_gated_mix__ssm_conv_h3__memory_aug_recurrent_mem_tr__prompt_kernel(
    A_q, A_k, A_v, A_shift_k, A_ssm_k, A_ssm_D, B_x, B_mem0,
    B_Wq, B_Wk, B_Wv, B_Wo, B_seg_len, gate_w,
):
    assert B_seg_len == SEG
    f32, bf16 = jnp.float32, jnp.bfloat16
    params = jnp.concatenate(
        [A_shift_k.T.astype(f32), A_ssm_D.reshape(1, D).astype(f32),
         gate_w.reshape(1, D).astype(f32), jnp.zeros((2, D), f32)], axis=0)
    hbm = pl.BlockSpec(memory_space=pl.ANY)
    vmem = pl.BlockSpec(memory_space=pltpu.VMEM)
    out = pl.pallas_call(
        _kernel,
        out_shape=jax.ShapeDtypeStruct((S, D), bf16),
        in_specs=[vmem, vmem, vmem, vmem] + [hbm] * 10,
        out_specs=hbm,
        scratch_shapes=[
            pltpu.VMEM((S, D), bf16),
            pltpu.VMEM((S, D), bf16),
            pltpu.VMEM((S, 128), f32),
            pltpu.VMEM((3, NG, D // 2, GW), jnp.uint32),
            pltpu.VMEM((D // 128, H * DH, 128), bf16),
            pltpu.VMEM((3, D // 128, 128 * H, DH), bf16),
            pltpu.VMEM((2, S, CT), bf16),
            pltpu.VMEM((2, S, CT), bf16),
            pltpu.VMEM((2, CT, S), bf16),
            pltpu.VMEM((8 + S, CT), f32),
            pltpu.VMEM((S, CT), f32),
            pltpu.VMEM((CT, S), f32),
            pltpu.VMEM((32, 128, CT), f32),
            pltpu.VMEM((32, CT, 128), f32),
            pltpu.VMEM((16, 256, 256), bf16),
            pltpu.VMEM((16, 256, 256), bf16),
            pltpu.VMEM((4, 8, H * DH), f32),
            pltpu.SemaphoreType.DMA((3, 2)),
            pltpu.SemaphoreType.DMA((3,)),
            pltpu.SemaphoreType.DMA((3,)),
            pltpu.SemaphoreType.DMA((D // 128,)),
            pltpu.SemaphoreType.DMA(()),
        ],
        compiler_params=pltpu.CompilerParams(vmem_limit_bytes=112 * 1024 * 1024),
    )(
        params, B_mem0.reshape(M, D), jnp.asarray(_GF8, bf16), jnp.asarray(_GI8, bf16),
        A_q.reshape(S, D), A_k.reshape(S, D), A_v.reshape(S, D), A_ssm_k,
        B_Wq.reshape(D // 128, 128 * H, DH), B_Wk.reshape(D // 128, 128 * H, DH), B_Wv.reshape(D // 128, 128 * H, DH),
        B_Wo.reshape(H * DH, D), jnp.asarray(_F, bf16), jnp.asarray(_FT, bf16),
    )
    return out.reshape(1, S, D)
```

```python
import functools

import jax
import jax.numpy as jnp
import numpy as np
from jax.experimental import pallas as pl
from jax.experimental.pallas import tpu as pltpu

S, D = 2048, 1024
H, DH = 32, 128
M, SEG = 8, 32
NSEG = S // SEG
KS = 4
CT = 256
NCT = D // CT
GH = 4
NG = H // GH
GW = GH * DH
ROWS = 48
NFFT = 2 * S
LAG = 3


def _fft_constants():
    n1 = np.arange(16)
    k1 = np.arange(16)
    c = np.exp(-1j * np.pi * np.outer(2 * k1 + 1, n1) / 32.0)
    gf = np.concatenate([c.real, c.imag], axis=0)
    gi = np.concatenate([c.real.T, c.imag.T], axis=1) * (2.0 / NFFT)
    eye = np.eye(8)
    gf8 = np.kron(gf, eye)
    gi8 = np.kron(gi, eye)
    n2 = np.arange(128)
    k2 = np.arange(128)
    f = np.zeros((16, 256, 256))
    for a in range(16):
        m = np.exp(-2j * np.pi * np.outer(a + 0.5 + 32.0 * k2, n2) / NFFT)
        f[a] = np.block([[m.real, -m.imag], [m.imag, m.real]])
    ft = np.transpose(f, (0, 2, 1))
    pos = np.arange(128)
    perm = 32 * (pos // 32) + 4 * (pos % 8) + (pos // 8) % 4
    fp = f[:, :, np.concatenate([perm, 128 + perm])]
    fall = np.concatenate([fp, f, ft], axis=0)
    return gf8.astype(np.float32), gi8.astype(np.float32), fall.astype(np.float32)


_GF8, _GI8, _FALL = _fft_constants()


def _kernel(p_ref, mem0_ref, gf_ref, gi_ref,
            q_hbm, k_hbm, v_hbm, h_hbm, wq_hbm, wk_hbm, wv_hbm, wo_hbm, f_hbm,
            out_hbm,
            x_s, o_s, g_s, wqkv_s, wo_s, st_s, kin_s, vin_s, hin_s,
            kpad_s, vf_s, hf_s, a_s, ah_s, y_s, b_s, f_s, stash_s,
            sem_in, sem_st, sem_misc, sem_wo, sem_out):
    bf16, f32 = jnp.bfloat16, jnp.float32

    def tile_copies(i, slot):
        c0 = pl.multiple_of(i * CT, CT)
        return (
            pltpu.make_async_copy(k_hbm.at[:, pl.ds(c0, CT)], kin_s.at[slot], sem_in.at[0, slot]),
            pltpu.make_async_copy(v_hbm.at[:, pl.ds(c0, CT)], vin_s.at[slot], sem_in.at[1, slot]),
            pltpu.make_async_copy(h_hbm.at[pl.ds(c0, CT), :], hin_s.at[slot], sem_in.at[2, slot]),
        )

    misc = (
        pltpu.make_async_copy(f_hbm.at[0:32], f_s.at[0:32], sem_misc.at[0]),
        pltpu.make_async_copy(f_hbm.at[32:48], f_s.at[32:48], sem_misc.at[1]),
        pltpu.make_async_copy(q_hbm, x_s, sem_misc.at[2]),
    )
    w_srcs = (wq_hbm, wk_hbm, wv_hbm)

    def st_copy(m):
        src = w_srcs[m] if isinstance(m, int) else w_srcs[0]
        return pltpu.make_async_copy(src, st_s.at[m].bitcast(bf16), sem_st.at[m])

    def wo_copy(j):
        return pltpu.make_async_copy(wo_hbm.at[:, pl.ds(j * 128, 128)], wo_s.at[j], sem_wo.at[j])

    for c in tile_copies(0, 0)[:2]:
        c.start()

    gf = gf_ref[...]
    gi = gi_ref[...]
    kpad_s[:, 0:8, :] = jnp.zeros((CT // 128, 8, 128), f32)

    gate_w = p_ref[5:6, :]

    def gate_body(r, carry):
        r0 = pl.multiple_of(r * 128, 128)
        xf = x_s[pl.ds(r0, 128), :].astype(f32) * gate_w
        sm = jnp.sum(xf, axis=-1, keepdims=True)
        g = 1.0 / (1.0 + jnp.exp(-sm))
        g_s[pl.ds(r0, 128), :] = jnp.broadcast_to(g, (128, 128))
        return carry


    def branch_a(i, slot):
        c0 = pl.multiple_of(i * CT, CT)
        for c in tile_copies(i, slot)[:2]:
            c.wait()

        @pl.when(i == 0)
        def _():
            tile_copies(0, 0)[2].start()
            misc[0].start()

        def cvt_body(r, carry):
            r0 = pl.multiple_of(r * 256, 256)
            kf = kin_s[slot, pl.ds(r0, 256), :].astype(f32)
            vf = vin_s[slot, pl.ds(r0, 256), :].astype(f32)
            for c in range(CT // 128):
                kpad_s[c, pl.ds(8 + r0, 256), :] = kf[:, c * 128:(c + 1) * 128]
                vf_s[c, pl.ds(r0, 256), :] = vf[:, c * 128:(c + 1) * 128]
            return carry

        jax.lax.fori_loop(0, S // 256, cvt_body, 0)

        @pl.when(i == 0)
        def _():
            for c in tile_copies(1, 1):
                c.start()


        pt = p_ref[:, pl.ds(c0, CT)]
        taps = [pt[j:j + 1, :] for j in range(KS)]
        dvec = pt[4:5, :]

        def sload(ref, t0):
            return jnp.concatenate(
                [ref[c, pl.ds(t0, 8, stride=4), :] for c in range(CT // 128)], axis=1)

        for jj in range(8):
            outs = []
            for j in (2 * jj, 2 * jj + 1):
                blocks = []
                for n1 in range(16):
                    t0 = n1 * 128 + 32 * (j // 4) + j % 4
                    acc = sload(kpad_s, 8 + t0) * taps[0]
                    for t in range(1, KS):
                        acc = acc + sload(kpad_s, 8 + t0 - t) * taps[t]
                    blocks.append(acc * sload(vf_s, t0))
                rhs = jnp.concatenate(blocks, axis=0).astype(bf16)
                outs.append(jnp.dot(gf, rhs, preferred_element_type=f32))
            for ks in range(32):
                a_s[ks, jj * 16:(jj + 1) * 16, :] = jnp.concatenate(
                    [o[ks * 8:(ks + 1) * 8] for o in outs], axis=0).astype(bf16)

        @pl.when(i == 0)
        def _():
            misc[1].start()
            misc[2].start()

        tile_copies(i, slot)[2].wait()
        hf_s[...] = hin_s[slot].astype(f32)


        def h1_body(j, carry):
            j8 = pl.multiple_of(j * 16, 16)
            lo = hf_s[pl.ds(j8, 8), :]
            hi = hf_s[pl.ds(j8 + 8, 8), :]
            blocks = [jnp.concatenate([lo[:, n1 * 128:(n1 + 1) * 128],
                                       hi[:, n1 * 128:(n1 + 1) * 128]], axis=1)
                      for n1 in range(16)]
            rhs = jnp.concatenate(blocks, axis=0).astype(bf16)
            out = jnp.dot(gf, rhs, preferred_element_type=f32)
            for ks in range(32):
                ah_s[ks, pl.ds(j8, 16), :] = jnp.concatenate(
                    [out[ks * 8:(ks + 1) * 8, 0:128], out[ks * 8:(ks + 1) * 8, 128:256]],
                    axis=0).astype(bf16)
            return carry

        jax.lax.fori_loop(0, CT // 16, h1_body, 0, unroll=4)

        @pl.when(i == 0)
        def _():
            misc[0].wait()

        def s2_body(k1, carry):
            a = jnp.concatenate([a_s[k1], a_s[16 + k1]], axis=0)
            xs = jnp.dot(f_s[k1], a, preferred_element_type=f32)
            ah = jnp.concatenate([ah_s[k1], ah_s[16 + k1]], axis=1)
            hs = jax.lax.dot_general(f_s[16 + k1], ah, (((1,), (1,)), ((), ())),
                                     preferred_element_type=f32)
            xr, xi = xs[0:128], xs[128:256]
            hr, hi = hs[0:128] + dvec, hs[128:256]
            y_s[k1] = jnp.concatenate([xr * hr - xi * hi, xr * hi + xi * hr], axis=0).astype(bf16)
            return carry

        jax.lax.fori_loop(0, 16, s2_body, 0, unroll=4)

        @pl.when(i == 0)
        def _():
            for t in (2, 3):
                for c in tile_copies(t, t):
                    c.start()
            misc[1].wait()

        def s3_body(k1, carry):
            b = jnp.dot(f_s[32 + k1], y_s[k1], preferred_element_type=f32)
            b_s[k1] = b[0:128]
            b_s[16 + k1] = b[128:256]
            return carry

        jax.lax.fori_loop(0, 16, s3_body, 0, unroll=4)

        @pl.when(i == 0)
        def _():
            st_copy(0).start()
            misc[2].wait()
            jax.lax.fori_loop(0, S // 128, gate_body, 0)


        def inv_body(jj, carry):
            j16 = pl.multiple_of(jj * 16, 16)
            ys = []
            for u in range(2):
                rhs = jnp.concatenate(
                    [b_s[ks, pl.ds(j16 + 8 * u, 8), :] for ks in range(32)], axis=0).astype(bf16)
                ys.append(jnp.dot(gi, rhs, preferred_element_type=f32))
            for n1 in range(16):
                r0 = pl.multiple_of(n1 * 128 + j16, 16)
                y = jnp.concatenate([ys[0][n1 * 8:(n1 + 1) * 8], ys[1][n1 * 8:(n1 + 1) * 8]], axis=0)
                qv = x_s[pl.ds(r0, 16), pl.ds(c0, CT)].astype(f32)
                g = g_s[pl.ds(r0, 16), :]
                g = jnp.concatenate([g] * (CT // 128), axis=1)
                o_s[pl.ds(r0, 16), pl.ds(c0, CT)] = (g * (qv * y)).astype(bf16)
            return carry

        jax.lax.fori_loop(0, 8, inv_body, 0, unroll=2)

    def repack(m):
        s32 = st_s.at[m]

        def body(c, carry):
            r0 = pl.multiple_of(c * 64, 64)
            for hp in range(H // 2):
                w = s32[c, pl.ds(hp, 128, stride=16), :]
                lo = pltpu.bitcast(w << 16, f32).astype(bf16)
                hi = pltpu.bitcast(w & jnp.uint32(0xFFFF0000), f32).astype(bf16)
                for hh, val in ((2 * hp, lo), (2 * hp + 1, hi)):
                    g, e = hh // GH, hh % GH
                    wqkv_s[m, g, pl.ds(r0, 64), e * 128:(e + 1) * 128] = pltpu.bitcast(val, jnp.uint32)
            return carry

        jax.lax.fori_loop(0, D // 128, body, 0)

    def phase1(i, carry):
        branch_a(i, i)

        @pl.when(i == 0)
        def _():
            st_copy(1).start()

        @pl.when(i == 1)
        def _():
            st_copy(2).start()

        @pl.when(i == 2)
        def _():
            for j in range(D // 128):
                wo_copy(j).start()
            st_copy(0).wait()
            repack(0)

        return carry

    jax.lax.fori_loop(0, NCT, phase1, 0)

    def repack_rest(m, carry):
        st_copy(m).wait()
        repack(m)
        return carry

    jax.lax.fori_loop(1, 3, repack_rest, 0)
    for j in range(D // 128):
        wo_copy(j).wait()

    row = jax.lax.broadcasted_iota(jnp.int32, (ROWS, ROWS), 0)
    col = jax.lax.broadcasted_iota(jnp.int32, (ROWS, ROWS), 1)
    mask0 = ((col < M) | (col >= 16)) & ((row < 16) | (col <= row))
    mask1 = ((col < 16) | (col >= 24)) & ((row < M) | (col <= row))
    scale = DH ** -0.5

    def getw(m, g):
        return pltpu.bitcast(wqkv_s[m, g], bf16)

    def getwo(g):
        return jnp.concatenate([wo_s[j, g * GW:(g + 1) * GW, :] for j in range(D // 128)], axis=1)

    def attn(q, k, v, mask):
        outs = []
        for e in range(GH):
            sl = slice(e * 128, (e + 1) * 128)
            s = jax.lax.dot_general(q[:, sl], k[:, sl], (((1,), (1,)), ((), ())),
                                    preferred_element_type=f32)
            s = jnp.where(mask, s * scale, -1e9)
            mx = jnp.max(s, axis=-1, keepdims=True)
            ex = jnp.exp(s - mx)
            sm = jnp.sum(ex, axis=-1, keepdims=True)
            p = (ex / sm).astype(bf16)
            outs.append(jnp.dot(p, v[:, sl], preferred_element_type=f32))
        return jnp.concatenate(outs, axis=1)

    def out_copy(j):
        r0 = pl.multiple_of(j * 2 * SEG, 2 * SEG)
        return pltpu.make_async_copy(o_s.at[pl.ds(r0, 2 * SEG), :],
                                     out_hbm.at[pl.ds(r0, 2 * SEG), :], sem_out)

    def half_step(hb, even):
        ts, os_ = {}, {}
        acc = None
        for g in range(NG + LAG):
            cs = slice(g * GW, (g + 1) * GW)
            if g < NG:
                ts[g] = tuple(jnp.dot(hb, getw(m, g), preferred_element_type=f32) for m in range(3))
            if 1 <= g <= NG:
                a = g - 1
                ca = slice(a * GW, (a + 1) * GW)
                if even:
                    for m in range(3):
                        stash_s[m, :, ca] = ts[a][m][8:16]
                    q, k, v = (t.astype(bf16) for t in ts[a])
                    o = attn(q, k, v, mask0)
                    stash_s[3, :, ca] = o[40:48]
                    os_[a] = jnp.concatenate([o[0:8], o[16:40]], axis=0).astype(bf16)
                else:
                    q, k, v = (jnp.concatenate(
                        [jnp.concatenate([ts[a][m][0:8], stash_s[m, :, ca]], axis=0).astype(bf16),
                         ts[a][m].astype(bf16)], axis=0) for m in range(3))
                    o = attn(q, k, v, mask1)
                    os_[a] = jnp.concatenate([o[0:16], stash_s[3, :, ca], o[24:48]], axis=0).astype(bf16)
            if g >= LAG:
                d = jnp.dot(os_[g - LAG], getwo(g - LAG), preferred_element_type=f32)
                acc = d if acc is None else acc + d
        return acc

    def step(j, mem):
        r0 = pl.multiple_of(j * 2 * SEG, 2 * SEG)
        xa = x_s[pl.ds(r0, SEG), :]
        xb = x_s[pl.ds(r0 + SEG, 16), :].astype(f32)
        xc = x_s[pl.ds(r0 + SEG + 16, 16), :]
        hb = jnp.concatenate([jnp.concatenate([mem, xb[0:8]], axis=0).astype(bf16), xa], axis=0)
        acc0 = half_step(hb, True)
        hb = jnp.concatenate([jnp.concatenate([acc0[0:8], xb[8:16]], axis=0).astype(bf16), xc], axis=0)
        acc1 = half_step(hb, False)
        b = jnp.concatenate([acc0[8:32], acc1[16:24], acc1[8:16], acc1[24:48]], axis=0)
        gb = g_s[pl.ds(r0, 2 * SEG), :]
        gb = jnp.concatenate([gb] * (D // 128), axis=1)
        res = o_s[pl.ds(r0, 2 * SEG), :].astype(f32) + (1.0 - gb) * b
        o_s[pl.ds(r0, 2 * SEG), :] = res.astype(bf16)
        out_copy(j).start()
        return acc1[0:8]

    jax.lax.fori_loop(0, NSEG // 2, step, mem0_ref[...].astype(f32))
    pltpu.make_async_copy(o_s, out_hbm, sem_out).wait()


@functools.partial(jax.jit, static_argnames=("B_seg_len",))
def pallas_gated_mix__ssm_conv_h3__memory_aug_recurrent_mem_tr__prompt_kernel(
    A_q, A_k, A_v, A_shift_k, A_ssm_k, A_ssm_D, B_x, B_mem0,
    B_Wq, B_Wk, B_Wv, B_Wo, B_seg_len, gate_w,
):
    assert B_seg_len == SEG
    f32, bf16 = jnp.float32, jnp.bfloat16
    params = jnp.concatenate(
        [A_shift_k.T.astype(f32), A_ssm_D.reshape(1, D).astype(f32),
         gate_w.reshape(1, D).astype(f32), jnp.zeros((2, D), f32)], axis=0)
    hbm = pl.BlockSpec(memory_space=pl.ANY)
    vmem = pl.BlockSpec(memory_space=pltpu.VMEM)
    out = pl.pallas_call(
        _kernel,
        out_shape=jax.ShapeDtypeStruct((S, D), bf16),
        in_specs=[vmem, vmem, vmem, vmem] + [hbm] * 9,
        out_specs=hbm,
        scratch_shapes=[
            pltpu.VMEM((S, D), bf16),
            pltpu.VMEM((S, D), bf16),
            pltpu.VMEM((S, 128), f32),
            pltpu.VMEM((3, NG, D // 2, GW), jnp.uint32),
            pltpu.VMEM((D // 128, H * DH, 128), bf16),
            pltpu.VMEM((3, D // 128, 64 * H, DH), jnp.uint32),
            pltpu.VMEM((NCT, S, CT), bf16),
            pltpu.VMEM((NCT, S, CT), bf16),
            pltpu.VMEM((NCT, CT, S), bf16),
            pltpu.VMEM((CT // 128, 8 + S, 128), f32),
            pltpu.VMEM((CT // 128, S, 128), f32),
            pltpu.VMEM((CT, S), f32),
            pltpu.VMEM((32, 128, CT), bf16),
            pltpu.VMEM((32, CT, 128), bf16),
            pltpu.VMEM((16, 256, CT), bf16),
            pltpu.VMEM((32, 128, CT), f32),
            pltpu.VMEM((48, 256, 256), bf16),
            pltpu.VMEM((4, 8, H * DH), f32),
            pltpu.SemaphoreType.DMA((3, NCT)),
            pltpu.SemaphoreType.DMA((3,)),
            pltpu.SemaphoreType.DMA((3,)),
            pltpu.SemaphoreType.DMA((D // 128,)),
            pltpu.SemaphoreType.DMA(()),
        ],
        compiler_params=pltpu.CompilerParams(vmem_limit_bytes=112 * 1024 * 1024),
    )(
        params, B_mem0.reshape(M, D), jnp.asarray(_GF8, bf16), jnp.asarray(_GI8, bf16),
        A_q.reshape(S, D), A_k.reshape(S, D), A_v.reshape(S, D), A_ssm_k,
        B_Wq.reshape(D // 128, 128 * H, DH), B_Wk.reshape(D // 128, 128 * H, DH), B_Wv.reshape(D // 128, 128 * H, DH),
        B_Wo.reshape(H * DH, D), jnp.asarray(_FALL, bf16),
    )
    return out.reshape(1, S, D)
```

```python
import functools

import jax
import jax.numpy as jnp
import numpy as np
from jax.experimental import pallas as pl
from jax.experimental.pallas import tpu as pltpu

S, D = 2048, 1024
H, DH = 32, 128
M, SEG = 8, 32
NSEG = S // SEG
KS = 4
CT = 256
NCT = D // CT
GH = 4
NG = H // GH
GW = GH * DH
ROWS = 48
NFFT = 2 * S
LAG = 3


def _fft_constants():
    n1 = np.arange(16)
    k1 = np.arange(16)
    c = np.exp(-1j * np.pi * np.outer(2 * k1 + 1, n1) / 32.0)
    gf = np.concatenate([c.real, c.imag], axis=0)
    gi = np.concatenate([c.real.T, c.imag.T], axis=1) * (2.0 / NFFT)
    eye = np.eye(8)
    gf8 = np.kron(gf, eye)
    gi8 = np.kron(gi, eye)
    n2 = np.arange(128)
    k2 = np.arange(128)
    f = np.zeros((16, 256, 256))
    for a in range(16):
        m = np.exp(-2j * np.pi * np.outer(a + 0.5 + 32.0 * k2, n2) / NFFT)
        f[a] = np.block([[m.real, -m.imag], [m.imag, m.real]])
    ft = np.transpose(f, (0, 2, 1))
    pos = np.arange(128)
    perm = 32 * (pos // 32) + 4 * (pos % 8) + (pos // 8) % 4
    fp = f[:, :, np.concatenate([perm, 128 + perm])]
    fall = np.concatenate([fp, f, ft], axis=0)
    return gf8.astype(np.float32), gi8.astype(np.float32), fall.astype(np.float32)


_GF8, _GI8, _FALL = _fft_constants()


def _kernel(p_ref, mem0_ref, gf_ref, gi_ref,
            q_hbm, k_hbm, v_hbm, h_hbm, wq_hbm, wk_hbm, wv_hbm, wo_hbm, f_hbm,
            out_hbm,
            x_s, o_s, wqkv_s, wo_s, st_s, kin_s, vin_s, hin_s,
            kpad_s, vf_s, hf_s, a_s, ah_s, y_s, b_s, f_s, stash_s,
            sem_in, sem_st, sem_misc, sem_wo, sem_out):
    bf16, f32 = jnp.bfloat16, jnp.float32

    def tile_copies(i, slot):
        c0 = pl.multiple_of(i * CT, CT)
        return (
            pltpu.make_async_copy(k_hbm.at[:, pl.ds(c0, CT)], kin_s.at[slot], sem_in.at[0, slot]),
            pltpu.make_async_copy(v_hbm.at[:, pl.ds(c0, CT)], vin_s.at[slot], sem_in.at[1, slot]),
            pltpu.make_async_copy(h_hbm.at[pl.ds(c0, CT), :], hin_s.at[slot], sem_in.at[2, slot]),
        )

    misc = (
        pltpu.make_async_copy(f_hbm.at[0:32], f_s.at[0:32], sem_misc.at[0]),
        pltpu.make_async_copy(f_hbm.at[32:48], f_s.at[32:48], sem_misc.at[1]),
        pltpu.make_async_copy(q_hbm, x_s, sem_misc.at[2]),
    )
    w_srcs = (wq_hbm, wk_hbm, wv_hbm)

    def st_copy(m):
        src = w_srcs[m] if isinstance(m, int) else w_srcs[0]
        return pltpu.make_async_copy(src, st_s.at[m].bitcast(bf16), sem_st.at[m])

    def st_start(i):
        for m in range(1, 3):
            @pl.when(i == m)
            def _():
                st_copy(m).start()

    def wo_copy(j):
        return pltpu.make_async_copy(wo_hbm.at[:, pl.ds(j * 128, 128)], wo_s.at[j], sem_wo.at[j])

    for c in tile_copies(0, 0)[:2]:
        c.start()

    gf = gf_ref[...]
    gi = gi_ref[...]
    kpad_s[:, 0:8, :] = jnp.zeros((CT // 128, 8, 128), f32)

    def repack_chunk(m, c):
        r0 = pl.multiple_of(c * 64, 64)
        for hp in range(H // 2):
            w = st_s[m, c, pl.ds(hp, 128, stride=16), :]
            lo = pltpu.bitcast(w << 16, f32).astype(bf16)
            hi = pltpu.bitcast(w & jnp.uint32(0xFFFF0000), f32).astype(bf16)
            for hh, val in ((2 * hp, lo), (2 * hp + 1, hi)):
                g, e = hh // GH, hh % GH
                wqkv_s[m, g, pl.ds(r0, 64), e * 128:(e + 1) * 128] = pltpu.bitcast(val, jnp.uint32)

    def branch_a(i, first):
        slot = i
        c0 = pl.multiple_of(i * CT, CT)
        kc, vc, hc = tile_copies(i, slot)
        kc.wait()
        vc.wait()
        if first:
            hc.start()
            misc[0].start()

        def cvt_body(r, carry):
            r0 = pl.multiple_of(r * 256, 256)
            kf = kin_s[slot, pl.ds(r0, 256), :].astype(f32)
            vf = vin_s[slot, pl.ds(r0, 256), :].astype(f32)
            for c in range(CT // 128):
                kpad_s[c, pl.ds(8 + r0, 256), :] = kf[:, c * 128:(c + 1) * 128]
                vf_s[c, pl.ds(r0, 256), :] = vf[:, c * 128:(c + 1) * 128]
            return carry

        jax.lax.fori_loop(0, S // 256, cvt_body, 0)

        if first:
            misc[1].start()
            for c in tile_copies(1, 1):
                c.start()

        pt = p_ref[:, pl.ds(c0, CT)]
        taps = [pt[j:j + 1, :] for j in range(KS)]
        dvec = pt[4:5, :]

        def sload(ref, t0):
            return jnp.concatenate(
                [ref[c, pl.ds(t0, 8, stride=4), :] for c in range(CT // 128)], axis=1)

        for jj in range(8):
            outs = []
            for j in (2 * jj, 2 * jj + 1):
                blocks = []
                for n1 in range(16):
                    t0 = n1 * 128 + 32 * (j // 4) + j % 4
                    acc = sload(kpad_s, 8 + t0) * taps[0]
                    for t in range(1, KS):
                        acc = acc + sload(kpad_s, 8 + t0 - t) * taps[t]
                    blocks.append(acc * sload(vf_s, t0))
                rhs = jnp.concatenate(blocks, axis=0).astype(bf16)
                outs.append(jnp.dot(gf, rhs, preferred_element_type=f32))
            for ks in range(32):
                a_s[ks, jj * 16:(jj + 1) * 16, :] = jnp.concatenate(
                    [o[ks * 8:(ks + 1) * 8] for o in outs], axis=0).astype(bf16)

        if not first:
            st_start(i)

        hc.wait()
        hf_s[...] = hin_s[slot].astype(f32)


        def h1_body(j, carry):
            j8 = pl.multiple_of(j * 16, 16)
            lo = hf_s[pl.ds(j8, 8), :]
            hi = hf_s[pl.ds(j8 + 8, 8), :]
            blocks = [jnp.concatenate([lo[:, n1 * 128:(n1 + 1) * 128],
                                       hi[:, n1 * 128:(n1 + 1) * 128]], axis=1)
                      for n1 in range(16)]
            rhs = jnp.concatenate(blocks, axis=0).astype(bf16)
            out = jnp.dot(gf, rhs, preferred_element_type=f32)
            for ks in range(32):
                ah_s[ks, pl.ds(j8, 16), :] = jnp.concatenate(
                    [out[ks * 8:(ks + 1) * 8, 0:128], out[ks * 8:(ks + 1) * 8, 128:256]],
                    axis=0).astype(bf16)
            return carry

        jax.lax.fori_loop(0, CT // 16, h1_body, 0, unroll=4)

        if first:
            misc[0].wait()
        else:
            st_copy(i - 1).wait()

        def s2_body(k1):
            a = jnp.concatenate([a_s[k1], a_s[16 + k1]], axis=0)
            xs = jnp.dot(f_s[k1], a, preferred_element_type=f32)
            ah = jnp.concatenate([ah_s[k1], ah_s[16 + k1]], axis=1)
            hs = jax.lax.dot_general(f_s[16 + k1], ah, (((1,), (1,)), ((), ())),
                                     preferred_element_type=f32)
            xr, xi = xs[0:128], xs[128:256]
            hr, hi = hs[0:128] + dvec, hs[128:256]
            y_s[k1] = jnp.concatenate([xr * hr - xi * hi, xr * hi + xi * hr], axis=0).astype(bf16)

        def s2_trip(t, carry):
            for u in range(4):
                s2_body(t * 4 + u)
            if not first:
                repack_chunk(i - 1, t)
            return carry

        jax.lax.fori_loop(0, 4, s2_trip, 0)

        if first:
            st_copy(0).start()
            misc[1].wait()

        def s3_body(k1):
            b = jnp.dot(f_s[32 + k1], y_s[k1], preferred_element_type=f32)
            b_s[k1] = b[0:128]
            b_s[16 + k1] = b[128:256]

        def s3_trip(t, carry):
            for u in range(4):
                s3_body(t * 4 + u)
            if not first:
                repack_chunk(i - 1, 4 + t)
            return carry

        jax.lax.fori_loop(0, 4, s3_trip, 0)

        def inv_body(jj, carry):
            j16 = pl.multiple_of(jj * 16, 16)
            ys = []
            for u in range(2):
                rhs = jnp.concatenate(
                    [b_s[ks, pl.ds(j16 + 8 * u, 8), :] for ks in range(32)], axis=0).astype(bf16)
                ys.append(jnp.dot(gi, rhs, preferred_element_type=f32))
            for n1 in range(16):
                r0 = pl.multiple_of(n1 * 128 + j16, 16)
                y = jnp.concatenate([ys[0][n1 * 8:(n1 + 1) * 8], ys[1][n1 * 8:(n1 + 1) * 8]], axis=0)
                o_s[pl.ds(r0, 16), pl.ds(c0, CT)] = y.astype(bf16)
            return carry

        jax.lax.fori_loop(0, 8, inv_body, 0, unroll=2)

        if first:
            for c in tile_copies(2, 2):
                c.start()
        else:
            @pl.when(i == 1)
            def _():
                for c in tile_copies(3, 3):
                    c.start()

            @pl.when(i == 2)
            def _():
                misc[2].start()
                for j in range(D // 128):
                    wo_copy(j).start()

    branch_a(0, True)

    def phase1(i, carry):
        branch_a(i, False)
        return carry

    jax.lax.fori_loop(1, NCT, phase1, 0)
    misc[2].wait()
    for j in range(D // 128):
        wo_copy(j).wait()

    row = jax.lax.broadcasted_iota(jnp.int32, (ROWS, ROWS), 0)
    col = jax.lax.broadcasted_iota(jnp.int32, (ROWS, ROWS), 1)
    mask0 = ((col < M) | (col >= 16)) & ((row < 16) | (col <= row))
    mask1 = ((col < 16) | (col >= 24)) & ((row < M) | (col <= row))
    scale = DH ** -0.5

    def getw(m, g):
        return pltpu.bitcast(wqkv_s[m, g], bf16)

    def getwo(g):
        return jnp.concatenate([wo_s[j, g * GW:(g + 1) * GW, :] for j in range(D // 128)], axis=1)

    def attn(q, k, v, mask):
        outs = []
        for e in range(GH):
            sl = slice(e * 128, (e + 1) * 128)
            s = jax.lax.dot_general(q[:, sl], k[:, sl], (((1,), (1,)), ((), ())),
                                    preferred_element_type=f32)
            s = jnp.where(mask, s * scale, -1e9)
            mx = jnp.max(s, axis=-1, keepdims=True)
            ex = jnp.exp(s - mx)
            sm = jnp.sum(ex, axis=-1, keepdims=True)
            p = (ex / sm).astype(bf16)
            outs.append(jnp.dot(p, v[:, sl], preferred_element_type=f32))
        return jnp.concatenate(outs, axis=1)

    def out_copy(j):
        r0 = pl.multiple_of(j * 2 * SEG, 2 * SEG)
        return pltpu.make_async_copy(o_s.at[pl.ds(r0, 2 * SEG), :],
                                     out_hbm.at[pl.ds(r0, 2 * SEG), :], sem_out)

    def half_step(hb, even):
        ts, os_ = {}, {}
        acc = None
        for g in range(NG + LAG):
            cs = slice(g * GW, (g + 1) * GW)
            if g < NG:
                ts[g] = tuple(jnp.dot(hb, getw(m, g), preferred_element_type=f32) for m in range(3))
            if 1 <= g <= NG:
                a = g - 1
                ca = slice(a * GW, (a + 1) * GW)
                if even:
                    for m in range(3):
                        stash_s[m, :, ca] = ts[a][m][8:16]
                    q, k, v = (t.astype(bf16) for t in ts[a])
                    o = attn(q, k, v, mask0)
                    stash_s[3, :, ca] = o[40:48]
                    os_[a] = jnp.concatenate([o[0:8], o[16:40]], axis=0).astype(bf16)
                else:
                    q, k, v = (jnp.concatenate(
                        [jnp.concatenate([ts[a][m][0:8], stash_s[m, :, ca]], axis=0).astype(bf16),
                         ts[a][m].astype(bf16)], axis=0) for m in range(3))
                    o = attn(q, k, v, mask1)
                    os_[a] = jnp.concatenate([o[0:16], stash_s[3, :, ca], o[24:48]], axis=0).astype(bf16)
            if g >= LAG:
                d = jnp.dot(os_[g - LAG], getwo(g - LAG), preferred_element_type=f32)
                acc = d if acc is None else acc + d
        return acc

    def step(j, mem):
        r0 = pl.multiple_of(j * 2 * SEG, 2 * SEG)
        xa = x_s[pl.ds(r0, SEG), :]
        xb = x_s[pl.ds(r0 + SEG, 16), :].astype(f32)
        xc = x_s[pl.ds(r0 + SEG + 16, 16), :]
        hb = jnp.concatenate([jnp.concatenate([mem, xb[0:8]], axis=0).astype(bf16), xa], axis=0)
        acc0 = half_step(hb, True)
        hb = jnp.concatenate([jnp.concatenate([acc0[0:8], xb[8:16]], axis=0).astype(bf16), xc], axis=0)
        acc1 = half_step(hb, False)
        b = jnp.concatenate([acc0[8:32], acc1[16:24], acc1[8:16], acc1[24:48]], axis=0)
        xf = x_s[pl.ds(r0, 2 * SEG), :].astype(f32)
        gate = jnp.sum(xf * p_ref[5:6, :], axis=-1, keepdims=True)
        gate = 1.0 / (1.0 + jnp.exp(-gate))
        res = gate * (xf * o_s[pl.ds(r0, 2 * SEG), :].astype(f32)) + (1.0 - gate) * b
        o_s[pl.ds(r0, 2 * SEG), :] = res.astype(bf16)
        out_copy(j).start()
        return acc1[0:8]

    jax.lax.fori_loop(0, NSEG // 2, step, mem0_ref[...].astype(f32))
    pltpu.make_async_copy(o_s, out_hbm, sem_out).wait()


@functools.partial(jax.jit, static_argnames=("B_seg_len",))
def pallas_gated_mix__ssm_conv_h3__memory_aug_recurrent_mem_tr__prompt_kernel(
    A_q, A_k, A_v, A_shift_k, A_ssm_k, A_ssm_D, B_x, B_mem0,
    B_Wq, B_Wk, B_Wv, B_Wo, B_seg_len, gate_w,
):
    assert B_seg_len == SEG
    f32, bf16 = jnp.float32, jnp.bfloat16
    params = jnp.concatenate(
        [A_shift_k.T.astype(f32), A_ssm_D.reshape(1, D).astype(f32),
         gate_w.reshape(1, D).astype(f32), jnp.zeros((2, D), f32)], axis=0)
    hbm = pl.BlockSpec(memory_space=pl.ANY)
    vmem = pl.BlockSpec(memory_space=pltpu.VMEM)
    out = pl.pallas_call(
        _kernel,
        out_shape=jax.ShapeDtypeStruct((S, D), bf16),
        in_specs=[vmem, vmem, vmem, vmem] + [hbm] * 9,
        out_specs=hbm,
        scratch_shapes=[
            pltpu.VMEM((S, D), bf16),
            pltpu.VMEM((S, D), bf16),
            pltpu.VMEM((3, NG, D // 2, GW), jnp.uint32),
            pltpu.VMEM((D // 128, H * DH, 128), bf16),
            pltpu.VMEM((3, D // 128, 64 * H, DH), jnp.uint32),
            pltpu.VMEM((NCT, S, CT), bf16),
            pltpu.VMEM((NCT, S, CT), bf16),
            pltpu.VMEM((NCT, CT, S), bf16),
            pltpu.VMEM((CT // 128, 8 + S, 128), f32),
            pltpu.VMEM((CT // 128, S, 128), f32),
            pltpu.VMEM((CT, S), f32),
            pltpu.VMEM((32, 128, CT), bf16),
            pltpu.VMEM((32, CT, 128), bf16),
            pltpu.VMEM((16, 256, CT), bf16),
            pltpu.VMEM((32, 128, CT), f32),
            pltpu.VMEM((48, 256, 256), bf16),
            pltpu.VMEM((4, 8, H * DH), f32),
            pltpu.SemaphoreType.DMA((3, NCT)),
            pltpu.SemaphoreType.DMA((3,)),
            pltpu.SemaphoreType.DMA((3,)),
            pltpu.SemaphoreType.DMA((D // 128,)),
            pltpu.SemaphoreType.DMA(()),
        ],
        compiler_params=pltpu.CompilerParams(vmem_limit_bytes=112 * 1024 * 1024),
    )(
        params, B_mem0.reshape(M, D), jnp.asarray(_GF8, bf16), jnp.asarray(_GI8, bf16),
        A_q.reshape(S, D), A_k.reshape(S, D), A_v.reshape(S, D), A_ssm_k,
        B_Wq.reshape(D // 128, 128 * H, DH), B_Wk.reshape(D // 128, 128 * H, DH), B_Wv.reshape(D // 128, 128 * H, DH),
        B_Wo.reshape(H * DH, D), jnp.asarray(_FALL, bf16),
    )
    return out.reshape(1, S, D)
```

```python
import functools

import jax
import jax.numpy as jnp
import numpy as np
from jax.experimental import pallas as pl
from jax.experimental.pallas import tpu as pltpu

S, D = 2048, 1024
H, DH = 32, 128
M, SEG = 8, 32
NSEG = S // SEG
KS = 4
CT = 256
NCT = D // CT
GH = 4
NG = H // GH
GW = GH * DH
ROWS = 48
NFFT = 2 * S
LAG = 3


def _fft_constants():
    n1 = np.arange(16)
    k1 = np.arange(16)
    c = np.exp(-1j * np.pi * np.outer(2 * k1 + 1, n1) / 32.0)
    gf = np.concatenate([c.real, c.imag], axis=0)
    gi = np.concatenate([c.real.T, c.imag.T], axis=1) * (2.0 / NFFT)
    eye = np.eye(8)
    gf8 = np.kron(gf, eye)
    gi8 = np.kron(gi, eye)
    n2 = np.arange(128)
    w = np.exp(-2j * np.pi * np.outer(n2, n2) / 128.0)
    tw = np.exp(-2j * np.pi * np.outer(np.arange(16) + 0.5, n2) / NFFT)
    perm = 32 * (n2 // 32) + 4 * (n2 % 8) + (n2 // 8) % 4
    cw = np.stack([w.real[:, perm], w.imag[:, perm], w.real, w.imag])
    ctw = np.stack([tw.real[:, perm], tw.imag[:, perm], tw.real, tw.imag])
    inv = []
    for a in range(16):
        m = np.conj(w * tw[a][None, :]).T
        inv += [m.real, m.imag, m.real + m.imag]
    return tuple(np.asarray(t, np.float32) for t in (gf8, gi8, cw, ctw, np.stack(inv)))


_GF8, _GI8, _CW, _CTW, _FINV = _fft_constants()


def _kernel(p_ref, mem0_ref, gf_ref, gi_ref, cw_ref, ctw_ref,
            q_hbm, k_hbm, v_hbm, h_hbm, wq_hbm, wk_hbm, wv_hbm, wo_hbm, f_hbm,
            out_hbm,
            x_s, o_s, wqkv_s, wo_s, st_s, kin_s, vin_s, hin_s,
            kpad_s, vf_s, hf_s, a_s, ah_s, y_s, b_s, f_s, stash_s,
            sem_in, sem_st, sem_misc, sem_wo, sem_out):
    bf16, f32 = jnp.bfloat16, jnp.float32

    def tile_copies(i, slot):
        c0 = pl.multiple_of(i * CT, CT)
        return (
            pltpu.make_async_copy(k_hbm.at[:, pl.ds(c0, CT)], kin_s.at[slot], sem_in.at[0, slot]),
            pltpu.make_async_copy(v_hbm.at[:, pl.ds(c0, CT)], vin_s.at[slot], sem_in.at[1, slot]),
            pltpu.make_async_copy(h_hbm.at[pl.ds(c0, CT), :], hin_s.at[slot], sem_in.at[2, slot]),
        )

    misc = (
        pltpu.make_async_copy(f_hbm, f_s.at[96:144], sem_misc.at[0]),
        pltpu.make_async_copy(q_hbm, x_s, sem_misc.at[1]),
    )
    w_srcs = (wq_hbm, wk_hbm, wv_hbm)

    def st_copy(m):
        src = w_srcs[m] if isinstance(m, int) else w_srcs[0]
        return pltpu.make_async_copy(src, st_s.at[m].bitcast(bf16), sem_st.at[m])

    def st_start(i):
        for m in range(1, 3):
            @pl.when(i == m)
            def _():
                st_copy(m).start()

    def wo_copy(j):
        return pltpu.make_async_copy(wo_hbm.at[:, pl.ds(j * 128, 128)], wo_s.at[j], sem_wo.at[j])

    for c in tile_copies(0, 0)[:2]:
        c.start()

    def build_f(a, carry):
        for v in range(2):
            wr, wi = cw_ref[2 * v], cw_ref[2 * v + 1]
            tr, ti = ctw_ref[2 * v, pl.ds(a, 1), :], ctw_ref[2 * v + 1, pl.ds(a, 1), :]
            mr = wr * tr - wi * ti
            mi = wr * ti + wi * tr
            f_s[v * 48 + 3 * a] = mr.astype(bf16)
            f_s[v * 48 + 3 * a + 1] = mi.astype(bf16)
            f_s[v * 48 + 3 * a + 2] = (mr + mi).astype(bf16)
        return carry

    jax.lax.fori_loop(0, 16, build_f, 0)
    gf = gf_ref[...]
    gi = gi_ref[...]
    kpad_s[:, 0:8, :] = jnp.zeros((CT // 128, 8, 128), f32)

    def repack_chunk(m, c, hps):
        r0 = pl.multiple_of(c * 64, 64)
        for hp in hps:
            w = st_s[m, c, pl.ds(hp, 128, stride=16), :]
            lo = pltpu.bitcast(w << 16, f32).astype(bf16)
            hi = pltpu.bitcast(w & jnp.uint32(0xFFFF0000), f32).astype(bf16)
            for hh, val in ((2 * hp, lo), (2 * hp + 1, hi)):
                g, e = hh // GH, hh % GH
                wqkv_s[m, g, pl.ds(r0, 64), e * 128:(e + 1) * 128] = pltpu.bitcast(val, jnp.uint32)

    def branch_a(i, first):
        slot = i
        c0 = pl.multiple_of(i * CT, CT)
        kc, vc, hc = tile_copies(i, slot)
        kc.wait()
        vc.wait()
        if first:
            hc.start()
            misc[0].start()
            for c in tile_copies(1, 1):
                c.start()

        def cvt_body(r, carry):
            r0 = pl.multiple_of(r * 256, 256)
            kf = kin_s[slot, pl.ds(r0, 256), :].astype(f32)
            vf = vin_s[slot, pl.ds(r0, 256), :].astype(f32)
            for c in range(CT // 128):
                kpad_s[c, pl.ds(8 + r0, 256), :] = kf[:, c * 128:(c + 1) * 128]
                vf_s[c, pl.ds(r0, 256), :] = vf[:, c * 128:(c + 1) * 128]
            return carry

        jax.lax.fori_loop(0, S // 256, cvt_body, 0)


        pt = p_ref[:, pl.ds(c0, CT)]
        taps = [pt[j:j + 1, :] for j in range(KS)]
        dvec = pt[4:5, :]

        def sload(ref, t0):
            return jnp.concatenate(
                [ref[c, pl.ds(t0, 8, stride=4), :] for c in range(CT // 128)], axis=1)

        for jj in range(8):
            outs = []
            for j in (2 * jj, 2 * jj + 1):
                blocks = []
                for n1 in range(16):
                    t0 = n1 * 128 + 32 * (j // 4) + j % 4
                    acc = sload(kpad_s, 8 + t0) * taps[0]
                    for t in range(1, KS):
                        acc = acc + sload(kpad_s, 8 + t0 - t) * taps[t]
                    blocks.append(acc * sload(vf_s, t0))
                rhs = jnp.concatenate(blocks, axis=0).astype(bf16)
                outs.append(jnp.dot(gf, rhs, preferred_element_type=f32))
            for ks in range(16):
                re, im = (jnp.concatenate([o[u * 8:(u + 1) * 8] for o in outs], axis=0)
                          for u in (ks, 16 + ks))
                for u, val in enumerate((re, im, re + im)):
                    a_s[3 * ks + u, jj * 16:(jj + 1) * 16, :] = val.astype(bf16)

        if not first:
            st_start(i)

        hc.wait()
        hf_s[...] = hin_s[slot].astype(f32)


        def h1_body(j, carry):
            j8 = pl.multiple_of(j * 16, 16)
            lo = hf_s[pl.ds(j8, 8), :]
            hi = hf_s[pl.ds(j8 + 8, 8), :]
            blocks = [jnp.concatenate([lo[:, n1 * 128:(n1 + 1) * 128],
                                       hi[:, n1 * 128:(n1 + 1) * 128]], axis=1)
                      for n1 in range(16)]
            rhs = jnp.concatenate(blocks, axis=0).astype(bf16)
            out = jnp.dot(gf, rhs, preferred_element_type=f32)
            for ks in range(16):
                re, im = (jnp.concatenate(
                    [out[u * 8:(u + 1) * 8, 0:128], out[u * 8:(u + 1) * 8, 128:256]], axis=0)
                    for u in (ks, 16 + ks))
                for u, val in enumerate((re, im, re + im)):
                    ah_s[3 * ks + u, pl.ds(j8, 16), :] = val.astype(bf16)
            return carry

        jax.lax.fori_loop(0, CT // 16, h1_body, 0, unroll=4)

        def cmul3(lhs, rhs, nt):
            dims = (((1,), (1,)), ((), ())) if nt else (((1,), (0,)), ((), ()))
            t1, t2, t3 = (jax.lax.dot_general(lhs(u), rhs(u), dims, preferred_element_type=f32)
                          for u in range(3))
            return t1 - t2, t3 - t1 - t2

        def s2_body(k1, carry):
            xr, xi = cmul3(lambda u: f_s[3 * k1 + u], lambda u: a_s[3 * k1 + u], False)
            hr, hi = cmul3(lambda u: f_s[48 + 3 * k1 + u], lambda u: ah_s[3 * k1 + u], True)
            hr = hr + dvec
            yr = xr * hr - xi * hi
            yi = xr * hi + xi * hr
            for u, val in enumerate((yr, yi, yr + yi)):
                y_s[3 * k1 + u] = val.astype(bf16)
            return carry

        jax.lax.fori_loop(0, 16, s2_body, 0, unroll=4)

        if first:
            st_copy(0).start()
            misc[0].wait()

        def s3_body(k1, carry):
            br, bi = cmul3(lambda u: f_s[96 + 3 * k1 + u], lambda u: y_s[3 * k1 + u], False)
            b_s[k1] = br
            b_s[16 + k1] = bi
            return carry

        jax.lax.fori_loop(0, 16, s3_body, 0, unroll=4)

        def inv_body(jj, carry):
            j16 = pl.multiple_of(jj * 16, 16)
            ys = []
            for u in range(2):
                rhs = jnp.concatenate(
                    [b_s[ks, pl.ds(j16 + 8 * u, 8), :] for ks in range(32)], axis=0).astype(bf16)
                ys.append(jnp.dot(gi, rhs, preferred_element_type=f32))
            for n1 in range(16):
                r0 = pl.multiple_of(n1 * 128 + j16, 16)
                y = jnp.concatenate([ys[0][n1 * 8:(n1 + 1) * 8], ys[1][n1 * 8:(n1 + 1) * 8]], axis=0)
                o_s[pl.ds(r0, 16), pl.ds(c0, CT)] = y.astype(bf16)
            return carry

        jax.lax.fori_loop(0, 8, inv_body, 0, unroll=2)

        if first:
            for c in tile_copies(2, 2):
                c.start()
        else:
            st_copy(i - 1).wait()

            def repack(c, carry):
                repack_chunk(i - 1, c, range(H // 2))
                return carry

            jax.lax.fori_loop(0, D // 128, repack, 0)

            @pl.when(i == 1)
            def _():
                for c in tile_copies(3, 3):
                    c.start()

            @pl.when(i == 2)
            def _():
                misc[1].start()
                for j in range(D // 128):
                    wo_copy(j).start()

    branch_a(0, True)

    def phase1(i, carry):
        branch_a(i, False)
        return carry

    jax.lax.fori_loop(1, NCT, phase1, 0)
    misc[1].wait()
    for j in range(D // 128):
        wo_copy(j).wait()

    row = jax.lax.broadcasted_iota(jnp.int32, (ROWS, ROWS), 0)
    col = jax.lax.broadcasted_iota(jnp.int32, (ROWS, ROWS), 1)
    mask0 = ((col < M) | (col >= 16)) & ((row < 16) | (col <= row))
    mask1 = ((col < 16) | (col >= 24)) & ((row < M) | (col <= row))
    scale = DH ** -0.5

    def getw(m, g):
        return pltpu.bitcast(wqkv_s[m, g], bf16)

    def getwo(g):
        return jnp.concatenate([wo_s[j, g * GW:(g + 1) * GW, :] for j in range(D // 128)], axis=1)

    def attn(q, k, v, mask):
        outs = []
        for e in range(GH):
            sl = slice(e * 128, (e + 1) * 128)
            s = jax.lax.dot_general(q[:, sl], k[:, sl], (((1,), (1,)), ((), ())),
                                    preferred_element_type=f32)
            s = jnp.where(mask, s * scale, -1e9)
            mx = jnp.max(s, axis=-1, keepdims=True)
            ex = jnp.exp(s - mx)
            sm = jnp.sum(ex, axis=-1, keepdims=True)
            p = (ex / sm).astype(bf16)
            outs.append(jnp.dot(p, v[:, sl], preferred_element_type=f32))
        return jnp.concatenate(outs, axis=1)

    def out_copy(j):
        r0 = pl.multiple_of(j * 2 * SEG, 2 * SEG)
        return pltpu.make_async_copy(o_s.at[pl.ds(r0, 2 * SEG), :],
                                     out_hbm.at[pl.ds(r0, 2 * SEG), :], sem_out)

    def half_step(hb, even):
        ts, os_ = {}, {}
        acc = None
        for g in range(NG + LAG):
            cs = slice(g * GW, (g + 1) * GW)
            if g < NG:
                ts[g] = tuple(jnp.dot(hb, getw(m, g), preferred_element_type=f32) for m in range(3))
            if 1 <= g <= NG:
                a = g - 1
                ca = slice(a * GW, (a + 1) * GW)
                if even:
                    for m in range(3):
                        stash_s[m, :, ca] = ts[a][m][8:16]
                    q, k, v = (t.astype(bf16) for t in ts[a])
                    o = attn(q, k, v, mask0)
                    stash_s[3, :, ca] = o[40:48]
                    os_[a] = jnp.concatenate([o[0:8], o[16:40]], axis=0).astype(bf16)
                else:
                    q, k, v = (jnp.concatenate(
                        [jnp.concatenate([ts[a][m][0:8], stash_s[m, :, ca]], axis=0).astype(bf16),
                         ts[a][m].astype(bf16)], axis=0) for m in range(3))
                    o = attn(q, k, v, mask1)
                    os_[a] = jnp.concatenate([o[0:16], stash_s[3, :, ca], o[24:48]], axis=0).astype(bf16)
            if g >= LAG:
                d = jnp.dot(os_[g - LAG], getwo(g - LAG), preferred_element_type=f32)
                acc = d if acc is None else acc + d
        return acc

    def step(j, mem):
        r0 = pl.multiple_of(j * 2 * SEG, 2 * SEG)
        xa = x_s[pl.ds(r0, SEG), :]
        xb = x_s[pl.ds(r0 + SEG, 16), :].astype(f32)
        xc = x_s[pl.ds(r0 + SEG + 16, 16), :]
        hb = jnp.concatenate([jnp.concatenate([mem, xb[0:8]], axis=0).astype(bf16), xa], axis=0)
        acc0 = half_step(hb, True)
        hb = jnp.concatenate([jnp.concatenate([acc0[0:8], xb[8:16]], axis=0).astype(bf16), xc], axis=0)
        acc1 = half_step(hb, False)
        b = jnp.concatenate([acc0[8:32], acc1[16:24], acc1[8:16], acc1[24:48]], axis=0)
        xf = x_s[pl.ds(r0, 2 * SEG), :].astype(f32)
        gate = jnp.sum(xf * p_ref[5:6, :], axis=-1, keepdims=True)
        gate = 1.0 / (1.0 + jnp.exp(-gate))
        res = gate * (xf * o_s[pl.ds(r0, 2 * SEG), :].astype(f32)) + (1.0 - gate) * b
        o_s[pl.ds(r0, 2 * SEG), :] = res.astype(bf16)
        out_copy(j).start()
        return acc1[0:8]

    jax.lax.fori_loop(0, NSEG // 2, step, mem0_ref[...].astype(f32))
    pltpu.make_async_copy(o_s, out_hbm, sem_out).wait()


@functools.partial(jax.jit, static_argnames=("B_seg_len",))
def pallas_gated_mix__ssm_conv_h3__memory_aug_recurrent_mem_tr__prompt_kernel(
    A_q, A_k, A_v, A_shift_k, A_ssm_k, A_ssm_D, B_x, B_mem0,
    B_Wq, B_Wk, B_Wv, B_Wo, B_seg_len, gate_w,
):
    assert B_seg_len == SEG
    f32, bf16 = jnp.float32, jnp.bfloat16
    params = jnp.concatenate(
        [A_shift_k.T.astype(f32), A_ssm_D.reshape(1, D).astype(f32),
         gate_w.reshape(1, D).astype(f32), jnp.zeros((2, D), f32)], axis=0)
    hbm = pl.BlockSpec(memory_space=pl.ANY)
    vmem = pl.BlockSpec(memory_space=pltpu.VMEM)
    out = pl.pallas_call(
        _kernel,
        out_shape=jax.ShapeDtypeStruct((S, D), bf16),
        in_specs=[vmem] * 6 + [hbm] * 9,
        out_specs=hbm,
        scratch_shapes=[
            pltpu.VMEM((S, D), bf16),
            pltpu.VMEM((S, D), bf16),
            pltpu.VMEM((3, NG, D // 2, GW), jnp.uint32),
            pltpu.VMEM((D // 128, H * DH, 128), bf16),
            pltpu.VMEM((3, D // 128, 64 * H, DH), jnp.uint32),
            pltpu.VMEM((NCT, S, CT), bf16),
            pltpu.VMEM((NCT, S, CT), bf16),
            pltpu.VMEM((NCT, CT, S), bf16),
            pltpu.VMEM((CT // 128, 8 + S, 128), f32),
            pltpu.VMEM((CT // 128, S, 128), f32),
            pltpu.VMEM((CT, S), f32),
            pltpu.VMEM((48, 128, CT), bf16),
            pltpu.VMEM((48, CT, 128), bf16),
            pltpu.VMEM((48, 128, CT), bf16),
            pltpu.VMEM((32, 128, CT), f32),
            pltpu.VMEM((144, 128, 128), bf16),
            pltpu.VMEM((4, 8, H * DH), f32),
            pltpu.SemaphoreType.DMA((3, NCT)),
            pltpu.SemaphoreType.DMA((3,)),
            pltpu.SemaphoreType.DMA((2,)),
            pltpu.SemaphoreType.DMA((D // 128,)),
            pltpu.SemaphoreType.DMA(()),
        ],
        compiler_params=pltpu.CompilerParams(vmem_limit_bytes=112 * 1024 * 1024),
    )(
        params, B_mem0.reshape(M, D), jnp.asarray(_GF8, bf16), jnp.asarray(_GI8, bf16),
        jnp.asarray(_CW), jnp.asarray(_CTW),
        A_q.reshape(S, D), A_k.reshape(S, D), A_v.reshape(S, D), A_ssm_k,
        B_Wq.reshape(D // 128, 128 * H, DH), B_Wk.reshape(D // 128, 128 * H, DH), B_Wv.reshape(D // 128, 128 * H, DH),
        B_Wo.reshape(H * DH, D), jnp.asarray(_FINV, bf16),
    )
    return out.reshape(1, S, D)
```

```python
import functools

import jax
import jax.numpy as jnp
import numpy as np
from jax.experimental import pallas as pl
from jax.experimental.pallas import tpu as pltpu

S, D = 2048, 1024
H, DH = 32, 128
M, SEG = 8, 32
NSEG = S // SEG
KS = 4
CT = 256
NCT = D // CT
GH = 4
NG = H // GH
GW = GH * DH
ROWS = 48
NFFT = 2 * S
LAG = 2


def _fft_constants():
    n1 = np.arange(16)
    k1 = np.arange(16)
    c = np.exp(-1j * np.pi * np.outer(2 * k1 + 1, n1) / 32.0)
    gf = np.concatenate([c.real, c.imag], axis=0)
    gi = np.concatenate([c.real.T, c.imag.T], axis=1) * (2.0 / NFFT)
    eye = np.eye(8)
    gf8 = np.kron(gf, eye)
    gi8 = np.kron(gi, eye)
    n2 = np.arange(128)
    w = np.exp(-2j * np.pi * np.outer(n2, n2) / 128.0)
    tw = np.exp(-2j * np.pi * np.outer(np.arange(16) + 0.5, n2) / NFFT)
    perm = 32 * (n2 // 32) + 4 * (n2 % 8) + (n2 // 8) % 4
    cw = np.stack([w.real[:, perm], w.imag[:, perm], w.real, w.imag])
    ctw = np.stack([tw.real[:, perm], tw.imag[:, perm], tw.real, tw.imag])
    inv = []
    for a in range(16):
        m = np.conj(w * tw[a][None, :]).T
        inv += [m.real, m.imag, m.real + m.imag]
    return tuple(np.asarray(t, np.float32) for t in (gf8, gi8, cw, ctw, np.stack(inv)))


_GF8, _GI8, _CW, _CTW, _FINV = _fft_constants()


def _kernel(taps_ref, d_ref, gw_ref, mem0_ref, gf_ref, gi_ref, cw_ref, ctw_ref,
            q_hbm, k_hbm, v_hbm, h_hbm, wq_hbm, wk_hbm, wv_hbm, wo_hbm, f_hbm,
            out_hbm,
            x_s, o_s, wqkv_s, wo_s, st_s, kin_s, vin_s, hin_s,
            kpad_s, vf_s, hf_s, a_s, ah_s, y_s, b_s, f_s, stash_s, par_s,
            sem_in, sem_st, sem_misc, sem_wo, sem_out):
    bf16, f32 = jnp.bfloat16, jnp.float32

    def k_copy(i):
        c0 = pl.multiple_of(i * CT, CT)
        return pltpu.make_async_copy(k_hbm.at[:, pl.ds(c0, CT)], kin_s.at[i], sem_in.at[0, i])

    def v_copy(i):
        c0 = pl.multiple_of(i * CT, CT)
        return pltpu.make_async_copy(v_hbm.at[:, pl.ds(c0, CT)], vin_s.at[i], sem_in.at[1, i])

    def h_copy(i):
        c0 = pl.multiple_of(i * CT, CT)
        return pltpu.make_async_copy(h_hbm.at[pl.ds(c0, CT), :], hin_s.at[i], sem_in.at[2, i])

    def start_tile(i):
        k_copy(i).start()
        v_copy(i).start()
        h_copy(i).start()

    misc = (
        pltpu.make_async_copy(f_hbm, f_s.at[96:144], sem_misc.at[0]),
        pltpu.make_async_copy(q_hbm, x_s, sem_misc.at[1]),
    )
    w_srcs = (wq_hbm, wk_hbm, wv_hbm)

    def st_copy(m):
        src = w_srcs[m] if isinstance(m, int) else w_srcs[0]
        return pltpu.make_async_copy(src, st_s.at[m].bitcast(bf16), sem_st.at[m])

    def st_start(i):
        for m in range(1, 3):
            @pl.when(i == m)
            def _():
                st_copy(m).start()

    def wo_copy(j):
        return pltpu.make_async_copy(wo_hbm.at[:, pl.ds(j * 128, 128)], wo_s.at[j], sem_wo.at[j])

    k_copy(0).start()
    v_copy(0).start()

    def build_f(a, carry):
        for v in range(2):
            wr, wi = cw_ref[2 * v], cw_ref[2 * v + 1]
            tr, ti = ctw_ref[2 * v, pl.ds(a, 1), :], ctw_ref[2 * v + 1, pl.ds(a, 1), :]
            mr = wr * tr - wi * ti
            mi = wr * ti + wi * tr
            f_s[v * 48 + 3 * a] = mr.astype(bf16)
            f_s[v * 48 + 3 * a + 1] = mi.astype(bf16)
            f_s[v * 48 + 3 * a + 2] = (mr + mi).astype(bf16)
        return carry

    jax.lax.fori_loop(0, 16, build_f, 0)
    par_s[...] = jnp.concatenate(
        [taps_ref[...].astype(f32), d_ref[...].astype(f32).reshape(1, D), gw_ref[...].astype(f32).reshape(1, D),
         jnp.zeros((2, D), f32)], axis=0)
    gf = gf_ref[...]
    gi = gi_ref[...]
    kpad_s[:, 0:8, :] = jnp.zeros((CT // 128, 8, 128), f32)

    def repack_chunk(m, c, hps):
        r0 = pl.multiple_of(c * 64, 64)
        for hp in hps:
            w = st_s[m, c, pl.ds(hp, 128, stride=16), :]
            lo = pltpu.bitcast(w << 16, f32).astype(bf16)
            hi = pltpu.bitcast(w & jnp.uint32(0xFFFF0000), f32).astype(bf16)
            for hh, val in ((2 * hp, lo), (2 * hp + 1, hi)):
                g, e = hh // GH, hh % GH
                wqkv_s[m, g, pl.ds(r0, 64), e * 128:(e + 1) * 128] = pltpu.bitcast(val, jnp.uint32)

    def branch_a(i, first):
        slot = i
        c0 = pl.multiple_of(i * CT, CT)
        k_copy(i).wait()
        v_copy(i).wait()
        if first:
            h_copy(0).start()
            misc[0].start()
            start_tile(1)

        def cvt_body(r, carry):
            r0 = pl.multiple_of(r * 256, 256)
            kf = kin_s[slot, pl.ds(r0, 256), :].astype(f32)
            vf = vin_s[slot, pl.ds(r0, 256), :].astype(f32)
            for c in range(CT // 128):
                kpad_s[c, pl.ds(8 + r0, 256), :] = kf[:, c * 128:(c + 1) * 128]
                vf_s[c, pl.ds(r0, 256), :] = vf[:, c * 128:(c + 1) * 128]
            return carry

        jax.lax.fori_loop(0, S // 256, cvt_body, 0)


        pt = par_s[:, pl.ds(c0, CT)]
        taps = [pt[j:j + 1, :] for j in range(KS)]
        dvec = pt[4:5, :]

        def sload(ref, t0):
            return jnp.concatenate(
                [ref[c, pl.ds(t0, 8, stride=4), :] for c in range(CT // 128)], axis=1)

        for jj in range(8):
            outs = []
            for j in (2 * jj, 2 * jj + 1):
                blocks = []
                for n1 in range(16):
                    t0 = n1 * 128 + 32 * (j // 4) + j % 4
                    acc = sload(kpad_s, 8 + t0) * taps[0]
                    for t in range(1, KS):
                        acc = acc + sload(kpad_s, 8 + t0 - t) * taps[t]
                    blocks.append(acc * sload(vf_s, t0))
                rhs = jnp.concatenate(blocks, axis=0).astype(bf16)
                outs.append(jnp.dot(gf, rhs, preferred_element_type=f32))
            for ks in range(16):
                re, im = (jnp.concatenate([o[u * 8:(u + 1) * 8] for o in outs], axis=0)
                          for u in (ks, 16 + ks))
                for u, val in enumerate((re, im, re + im)):
                    a_s[3 * ks + u, jj * 16:(jj + 1) * 16, :] = val.astype(bf16)

        if not first:
            st_start(i)

        h_copy(i).wait()
        hf_s[...] = hin_s[slot].astype(f32)


        def h1_body(j, carry):
            j8 = pl.multiple_of(j * 16, 16)
            lo = hf_s[pl.ds(j8, 8), :]
            hi = hf_s[pl.ds(j8 + 8, 8), :]
            blocks = [jnp.concatenate([lo[:, n1 * 128:(n1 + 1) * 128],
                                       hi[:, n1 * 128:(n1 + 1) * 128]], axis=1)
                      for n1 in range(16)]
            rhs = jnp.concatenate(blocks, axis=0).astype(bf16)
            out = jnp.dot(gf, rhs, preferred_element_type=f32)
            for ks in range(16):
                re, im = (jnp.concatenate(
                    [out[u * 8:(u + 1) * 8, 0:128], out[u * 8:(u + 1) * 8, 128:256]], axis=0)
                    for u in (ks, 16 + ks))
                for u, val in enumerate((re, im, re + im)):
                    ah_s[3 * ks + u, pl.ds(j8, 16), :] = val.astype(bf16)
            return carry

        jax.lax.fori_loop(0, CT // 16, h1_body, 0, unroll=4)

        def cmul3(lhs, rhs, nt):
            dims = (((1,), (1,)), ((), ())) if nt else (((1,), (0,)), ((), ()))
            t1, t2, t3 = (jax.lax.dot_general(lhs(u), rhs(u), dims, preferred_element_type=f32)
                          for u in range(3))
            return t1 - t2, t3 - t1 - t2

        def s2_body(k1, carry):
            xr, xi = cmul3(lambda u: f_s[3 * k1 + u], lambda u: a_s[3 * k1 + u], False)
            hr, hi = cmul3(lambda u: f_s[48 + 3 * k1 + u], lambda u: ah_s[3 * k1 + u], True)
            hr = hr + dvec
            yr = xr * hr - xi * hi
            yi = xr * hi + xi * hr
            for u, val in enumerate((yr, yi, yr + yi)):
                y_s[3 * k1 + u] = val.astype(bf16)
            return carry

        jax.lax.fori_loop(0, 16, s2_body, 0, unroll=4)

        if first:
            st_copy(0).start()
            misc[0].wait()

        def s3_body(k1, carry):
            br, bi = cmul3(lambda u: f_s[96 + 3 * k1 + u], lambda u: y_s[3 * k1 + u], False)
            b_s[k1] = br
            b_s[16 + k1] = bi
            return carry

        jax.lax.fori_loop(0, 16, s3_body, 0, unroll=4)

        def inv_body(jj, carry):
            j16 = pl.multiple_of(jj * 16, 16)
            ys = []
            for u in range(2):
                rhs = jnp.concatenate(
                    [b_s[ks, pl.ds(j16 + 8 * u, 8), :] for ks in range(32)], axis=0).astype(bf16)
                ys.append(jnp.dot(gi, rhs, preferred_element_type=f32))
            for n1 in range(16):
                r0 = pl.multiple_of(n1 * 128 + j16, 16)
                y = jnp.concatenate([ys[0][n1 * 8:(n1 + 1) * 8], ys[1][n1 * 8:(n1 + 1) * 8]], axis=0)
                o_s[pl.ds(r0, 16), pl.ds(c0, CT)] = y.astype(bf16)
            return carry

        jax.lax.fori_loop(0, 8, inv_body, 0, unroll=2)

        if first:
            start_tile(2)
        else:
            st_copy(i - 1).wait()

            def repack(c, carry):
                repack_chunk(i - 1, c, range(H // 2))
                return carry

            jax.lax.fori_loop(0, D // 128, repack, 0)

            @pl.when(i == 1)
            def _():
                start_tile(3)

            @pl.when(i == 2)
            def _():
                misc[1].start()
                for j in range(D // 128):
                    wo_copy(j).start()

    branch_a(0, True)

    def phase1(i, carry):
        branch_a(i, False)
        return carry

    jax.lax.fori_loop(1, NCT, phase1, 0)
    misc[1].wait()
    for j in range(D // 128):
        wo_copy(j).wait()

    row = jax.lax.broadcasted_iota(jnp.int32, (ROWS, ROWS), 0)
    col = jax.lax.broadcasted_iota(jnp.int32, (ROWS, ROWS), 1)
    mask0 = ((col < M) | (col >= 16)) & ((row < 16) | (col <= row))
    mask1 = ((col < 16) | (col >= 24)) & ((row < M) | (col <= row))
    scale = DH ** -0.5

    def getw(m, g):
        return pltpu.bitcast(wqkv_s[m, g], bf16)

    def getwo(g):
        return jnp.concatenate([wo_s[j, g * GW:(g + 1) * GW, :] for j in range(D // 128)], axis=1)

    def attn(q, k, v, mask):
        outs = []
        for e in range(GH):
            sl = slice(e * 128, (e + 1) * 128)
            s = jax.lax.dot_general(q[:, sl], k[:, sl], (((1,), (1,)), ((), ())),
                                    preferred_element_type=f32)
            s = jnp.where(mask, s * scale, -1e9)
            mx = jnp.max(s, axis=-1, keepdims=True)
            ex = jnp.exp(s - mx)
            sm = jnp.sum(ex, axis=-1, keepdims=True)
            p = (ex / sm).astype(bf16)
            outs.append(jnp.dot(p, v[:, sl], preferred_element_type=f32))
        return jnp.concatenate(outs, axis=1)

    def out_copy(j):
        r0 = pl.multiple_of(j * 2 * SEG, 2 * SEG)
        return pltpu.make_async_copy(o_s.at[pl.ds(r0, 2 * SEG), :],
                                     out_hbm.at[pl.ds(r0, 2 * SEG), :], sem_out)

    def half_step(hb, even):
        ts, os_ = {}, {}
        acc = None
        for g in range(NG + LAG):
            cs = slice(g * GW, (g + 1) * GW)
            if g < NG:
                ts[g] = tuple(jnp.dot(hb, getw(m, g), preferred_element_type=f32) for m in range(3))
            if 1 <= g <= NG:
                a = g - 1
                ca = slice(a * GW, (a + 1) * GW)
                if even:
                    for m in range(3):
                        stash_s[m, :, ca] = ts[a][m][8:16]
                    q, k, v = (t.astype(bf16) for t in ts[a])
                    o = attn(q, k, v, mask0)
                    stash_s[3, :, ca] = o[40:48]
                    os_[a] = jnp.concatenate([o[0:8], o[16:40]], axis=0).astype(bf16)
                else:
                    q, k, v = (jnp.concatenate(
                        [jnp.concatenate([ts[a][m][0:8], stash_s[m, :, ca]], axis=0).astype(bf16),
                         ts[a][m].astype(bf16)], axis=0) for m in range(3))
                    o = attn(q, k, v, mask1)
                    os_[a] = jnp.concatenate([o[0:16], stash_s[3, :, ca], o[24:48]], axis=0).astype(bf16)
            if g >= LAG:
                d = jnp.dot(os_[g - LAG], getwo(g - LAG), preferred_element_type=f32)
                acc = d if acc is None else acc + d
        return acc

    def step(j, mem):
        r0 = pl.multiple_of(j * 2 * SEG, 2 * SEG)
        xa = x_s[pl.ds(r0, SEG), :]
        xb = x_s[pl.ds(r0 + SEG, 16), :].astype(f32)
        xc = x_s[pl.ds(r0 + SEG + 16, 16), :]
        hb = jnp.concatenate([jnp.concatenate([mem, xb[0:8]], axis=0).astype(bf16), xa], axis=0)
        acc0 = half_step(hb, True)
        hb = jnp.concatenate([jnp.concatenate([acc0[0:8], xb[8:16]], axis=0).astype(bf16), xc], axis=0)
        acc1 = half_step(hb, False)
        b = jnp.concatenate([acc0[8:32], acc1[16:24], acc1[8:16], acc1[24:48]], axis=0)
        xf = x_s[pl.ds(r0, 2 * SEG), :].astype(f32)
        gate = jnp.sum(xf * par_s[5:6, :], axis=-1, keepdims=True)
        gate = 1.0 / (1.0 + jnp.exp(-gate))
        res = gate * (xf * o_s[pl.ds(r0, 2 * SEG), :].astype(f32)) + (1.0 - gate) * b
        o_s[pl.ds(r0, 2 * SEG), :] = res.astype(bf16)
        out_copy(j).start()
        return acc1[0:8]

    jax.lax.fori_loop(0, NSEG // 2, step, mem0_ref[...].astype(f32))
    pltpu.make_async_copy(o_s, out_hbm, sem_out).wait()


@functools.partial(jax.jit, static_argnames=("B_seg_len",))
def pallas_gated_mix__ssm_conv_h3__memory_aug_recurrent_mem_tr__prompt_kernel(
    A_q, A_k, A_v, A_shift_k, A_ssm_k, A_ssm_D, B_x, B_mem0,
    B_Wq, B_Wk, B_Wv, B_Wo, B_seg_len, gate_w,
):
    assert B_seg_len == SEG
    bf16 = jnp.bfloat16
    f32 = jnp.float32
    hbm = pl.BlockSpec(memory_space=pl.ANY)
    vmem = pl.BlockSpec(memory_space=pltpu.VMEM)
    out = pl.pallas_call(
        _kernel,
        out_shape=jax.ShapeDtypeStruct((S, D), bf16),
        in_specs=[vmem] * 8 + [hbm] * 9,
        out_specs=hbm,
        scratch_shapes=[
            pltpu.VMEM((S, D), bf16),
            pltpu.VMEM((S, D), bf16),
            pltpu.VMEM((3, NG, D // 2, GW), jnp.uint32),
            pltpu.VMEM((D // 128, H * DH, 128), bf16),
            pltpu.VMEM((3, D // 128, 64 * H, DH), jnp.uint32),
            pltpu.VMEM((NCT, S, CT), bf16),
            pltpu.VMEM((NCT, S, CT), bf16),
            pltpu.VMEM((NCT, CT, S), bf16),
            pltpu.VMEM((CT // 128, 8 + S, 128), f32),
            pltpu.VMEM((CT // 128, S, 128), f32),
            pltpu.VMEM((CT, S), f32),
            pltpu.VMEM((48, 128, CT), bf16),
            pltpu.VMEM((48, CT, 128), bf16),
            pltpu.VMEM((48, 128, CT), bf16),
            pltpu.VMEM((32, 128, CT), f32),
            pltpu.VMEM((144, 128, 128), bf16),
            pltpu.VMEM((4, 8, H * DH), f32),
            pltpu.VMEM((8, D), f32),
            pltpu.SemaphoreType.DMA((3, NCT)),
            pltpu.SemaphoreType.DMA((3,)),
            pltpu.SemaphoreType.DMA((2,)),
            pltpu.SemaphoreType.DMA((D // 128,)),
            pltpu.SemaphoreType.DMA(()),
        ],
        compiler_params=pltpu.CompilerParams(vmem_limit_bytes=112 * 1024 * 1024),
    )(
        A_shift_k.T, A_ssm_D, gate_w, B_mem0.reshape(M, D), jnp.asarray(_GF8, bf16), jnp.asarray(_GI8, bf16),
        jnp.asarray(_CW), jnp.asarray(_CTW),
        A_q.reshape(S, D), A_k.reshape(S, D), A_v.reshape(S, D), A_ssm_k,
        B_Wq.reshape(D // 128, 128 * H, DH), B_Wk.reshape(D // 128, 128 * H, DH), B_Wv.reshape(D // 128, 128 * H, DH),
        B_Wo.reshape(H * DH, D), jnp.asarray(_FINV, bf16),
    )
    return out.reshape(1, S, D)
```

```python
import functools

import jax
import jax.numpy as jnp
import numpy as np
from jax.experimental import pallas as pl
from jax.experimental.pallas import tpu as pltpu

S, D = 2048, 1024
H, DH = 32, 128
M, SEG = 8, 32
NSEG = S // SEG
KS = 4
CT = 256
NCT = D // CT
GH = 4
NG = H // GH
GW = GH * DH
ROWS = 48
NFFT = 2 * S
XH = 256
LAG = 2


def _fft_constants():
    n1 = np.arange(16)
    k1 = np.arange(16)
    c = np.exp(-1j * np.pi * np.outer(2 * k1 + 1, n1) / 32.0)
    gf = np.concatenate([c.real, c.imag], axis=0)
    gi = np.concatenate([c.real.T, c.imag.T], axis=1) * (2.0 / NFFT)
    eye = np.eye(8)
    gf8 = np.kron(gf, eye)
    gi8 = np.kron(gi, eye)
    n2 = np.arange(128)
    w = np.exp(-2j * np.pi * np.outer(n2, n2) / 128.0)
    tw = np.exp(-2j * np.pi * np.outer(np.arange(16) + 0.5, n2) / NFFT)
    perm = 32 * (n2 // 32) + 4 * (n2 % 8) + (n2 // 8) % 4
    cw = np.stack([w.real[:, perm], w.imag[:, perm], w.real, w.imag])
    ctw = np.stack([tw.real[:, perm], tw.imag[:, perm], tw.real, tw.imag])
    inv = []
    for a in range(16):
        m = np.conj(w * tw[a][None, :]).T
        inv += [m.real, m.imag, m.real + m.imag]
    return tuple(np.asarray(t, np.float32) for t in (gf8, gi8, cw, ctw, np.stack(inv)))


_GF8, _GI8, _CW, _CTW, _FINV = _fft_constants()


def _kernel(taps_ref, d_ref, gw_ref, mem0_ref, gf_ref, gi_ref, cw_ref, ctw_ref,
            q_hbm, k_hbm, v_hbm, h_hbm, wq_hbm, wk_hbm, wv_hbm, wo_hbm, f_hbm,
            out_hbm,
            x_s, o_s, wqkv_s, wo_s, st_s, kin_s, vin_s, hin_s,
            kpad_s, vf_s, a_s, ah_s, y_s, b_s, f_s, stash_s, par_s,
            sem_in, sem_st, sem_misc, sem_wo, sem_out):
    bf16, f32 = jnp.bfloat16, jnp.float32

    def k_copy(i):
        c0 = pl.multiple_of(i * CT, CT)
        return pltpu.make_async_copy(k_hbm.at[:, pl.ds(c0, CT)], kin_s.at[i], sem_in.at[0, i])

    def v_copy(i):
        c0 = pl.multiple_of(i * CT, CT)
        return pltpu.make_async_copy(v_hbm.at[:, pl.ds(c0, CT)], vin_s.at[i], sem_in.at[1, i])

    def h_copy(i):
        c0 = pl.multiple_of(i * CT, CT)
        return pltpu.make_async_copy(h_hbm.at[pl.ds(c0, CT), :], hin_s.at[i], sem_in.at[2, i])

    def start_tile(i):
        k_copy(i).start()
        v_copy(i).start()
        h_copy(i).start()

    misc = (
        pltpu.make_async_copy(f_hbm, f_s.at[96:144], sem_misc.at[0]),
        pltpu.make_async_copy(q_hbm.at[0:XH], x_s.at[0:XH], sem_misc.at[1]),
        pltpu.make_async_copy(q_hbm.at[XH:S], x_s.at[XH:S], sem_misc.at[2]),
    )
    w_srcs = (wq_hbm, wk_hbm, wv_hbm)

    def st_copy(m):
        src = w_srcs[m] if isinstance(m, int) else w_srcs[0]
        return pltpu.make_async_copy(src, st_s.at[m].bitcast(bf16), sem_st.at[m])

    def wo_copy(j):
        return pltpu.make_async_copy(wo_hbm.at[:, pl.ds(j * 128, 128)], wo_s.at[j], sem_wo.at[j])

    k_copy(0).start()
    v_copy(0).start()

    def build_f(a, carry):
        for v in range(2):
            wr, wi = cw_ref[2 * v], cw_ref[2 * v + 1]
            tr, ti = ctw_ref[2 * v, pl.ds(a, 1), :], ctw_ref[2 * v + 1, pl.ds(a, 1), :]
            mr = wr * tr - wi * ti
            mi = wr * ti + wi * tr
            f_s[v * 48 + 3 * a] = mr.astype(bf16)
            f_s[v * 48 + 3 * a + 1] = mi.astype(bf16)
            f_s[v * 48 + 3 * a + 2] = (mr + mi).astype(bf16)
        return carry

    jax.lax.fori_loop(0, 16, build_f, 0)
    par_s[...] = jnp.concatenate(
        [taps_ref[...].astype(f32), d_ref[...].astype(f32).reshape(1, D), gw_ref[...].astype(f32).reshape(1, D),
         jnp.zeros((2, D), f32)], axis=0)
    gf = gf_ref[...]
    gi = gi_ref[...]
    kpad_s[:, 0:8, :] = jnp.zeros((CT // 128, 8, 128), f32)

    def repack_chunk(m, c, hps):
        r0 = pl.multiple_of(c * 64, 64)
        for hp in hps:
            w = st_s[m, c, pl.ds(hp, 128, stride=16), :]
            lo = pltpu.bitcast(w << 16, f32).astype(bf16)
            hi = pltpu.bitcast(w & jnp.uint32(0xFFFF0000), f32).astype(bf16)
            for hh, val in ((2 * hp, lo), (2 * hp + 1, hi)):
                g, e = hh // GH, hh % GH
                wqkv_s[m, g, pl.ds(r0, 64), e * 128:(e + 1) * 128] = pltpu.bitcast(val, jnp.uint32)

    def branch_a(i, first):
        slot = i
        c0 = pl.multiple_of(i * CT, CT)
        k_copy(i).wait()
        v_copy(i).wait()
        if first:
            h_copy(0).start()
            misc[0].start()
            start_tile(1)

        def cvt_body(r, carry):
            r0 = pl.multiple_of(r * 256, 256)
            kf = kin_s[slot, pl.ds(r0, 256), :].astype(f32)
            vf = vin_s[slot, pl.ds(r0, 256), :].astype(f32)
            for c in range(CT // 128):
                kpad_s[c, pl.ds(8 + r0, 256), :] = kf[:, c * 128:(c + 1) * 128]
                vf_s[c, pl.ds(r0, 256), :] = vf[:, c * 128:(c + 1) * 128]
            return carry

        jax.lax.fori_loop(0, S // 256, cvt_body, 0)


        pt = par_s[:, pl.ds(c0, CT)]
        taps = [pt[j:j + 1, :] for j in range(KS)]
        dvec = pt[4:5, :]

        def sload(ref, t0):
            return jnp.concatenate(
                [ref[c, pl.ds(t0, 8, stride=4), :] for c in range(CT // 128)], axis=1)

        for jj in range(8):
            outs = []
            for j in (2 * jj, 2 * jj + 1):
                blocks = []
                for n1 in range(16):
                    t0 = n1 * 128 + 32 * (j // 4) + j % 4
                    acc = sload(kpad_s, 8 + t0) * taps[0]
                    for t in range(1, KS):
                        acc = acc + sload(kpad_s, 8 + t0 - t) * taps[t]
                    blocks.append(acc * sload(vf_s, t0))
                rhs = jnp.concatenate(blocks, axis=0).astype(bf16)
                outs.append(jnp.dot(gf, rhs, preferred_element_type=f32))
            for ks in range(16):
                re, im = (jnp.concatenate([o[u * 8:(u + 1) * 8] for o in outs], axis=0)
                          for u in (ks, 16 + ks))
                for u, val in enumerate((re, im, re + im)):
                    a_s[3 * ks + u, jj * 16:(jj + 1) * 16, :] = val.astype(bf16)

        if first:
            st_copy(0).start()
        else:
            @pl.when(i == 1)
            def _():
                start_tile(3)

            @pl.when(i == 2)
            def _():
                misc[1].start()
                for j in range(D // 128):
                    wo_copy(j).start()
                misc[2].start()

        h_copy(i).wait()


        def h1_body(j, carry):
            j8 = pl.multiple_of(j * 16, 16)
            hv = hin_s[slot, pl.ds(j8, 16), :].astype(f32)
            lo, hi = hv[0:8], hv[8:16]
            blocks = [jnp.concatenate([lo[:, n1 * 128:(n1 + 1) * 128],
                                       hi[:, n1 * 128:(n1 + 1) * 128]], axis=1)
                      for n1 in range(16)]
            rhs = jnp.concatenate(blocks, axis=0).astype(bf16)
            out = jnp.dot(gf, rhs, preferred_element_type=f32)
            for ks in range(16):
                re, im = (jnp.concatenate(
                    [out[u * 8:(u + 1) * 8, 0:128], out[u * 8:(u + 1) * 8, 128:256]], axis=0)
                    for u in (ks, 16 + ks))
                for u, val in enumerate((re, im, re + im)):
                    ah_s[3 * ks + u, pl.ds(j8, 16), :] = val.astype(bf16)
            return carry

        jax.lax.fori_loop(0, CT // 16, h1_body, 0, unroll=8)

        def cmul3(lhs, rhs, nt):
            dims = (((1,), (1,)), ((), ())) if nt else (((1,), (0,)), ((), ()))
            t1, t2, t3 = (jax.lax.dot_general(lhs(u), rhs(u), dims, preferred_element_type=f32)
                          for u in range(3))
            return t1 - t2, t3 - t1 - t2

        def s2_body(k1, carry):
            xr, xi = cmul3(lambda u: f_s[3 * k1 + u], lambda u: a_s[3 * k1 + u], False)
            hr, hi = cmul3(lambda u: f_s[48 + 3 * k1 + u], lambda u: ah_s[3 * k1 + u], True)
            hr = hr + dvec
            yr = xr * hr - xi * hi
            yi = xr * hi + xi * hr
            for u, val in enumerate((yr, yi, yr + yi)):
                y_s[3 * k1 + u] = val.astype(bf16)
            return carry

        jax.lax.fori_loop(0, 16, s2_body, 0, unroll=8)

        if first:
            start_tile(2)
            misc[0].wait()

        def s3_body(k1, carry):
            br, bi = cmul3(lambda u: f_s[96 + 3 * k1 + u], lambda u: y_s[3 * k1 + u], False)
            b_s[k1] = br
            b_s[16 + k1] = bi
            return carry

        jax.lax.fori_loop(0, 16, s3_body, 0, unroll=8)

        def inv_body(jj, carry):
            j16 = pl.multiple_of(jj * 16, 16)
            ys = []
            for u in range(2):
                rhs = jnp.concatenate(
                    [b_s[ks, pl.ds(j16 + 8 * u, 8), :] for ks in range(32)], axis=0).astype(bf16)
                ys.append(jnp.dot(gi, rhs, preferred_element_type=f32))
            for n1 in range(16):
                r0 = pl.multiple_of(n1 * 128 + j16, 16)
                y = jnp.concatenate([ys[0][n1 * 8:(n1 + 1) * 8], ys[1][n1 * 8:(n1 + 1) * 8]], axis=0)
                o_s[pl.ds(r0, 16), pl.ds(c0, CT)] = y.astype(bf16)
            return carry

        jax.lax.fori_loop(0, 8, inv_body, 0, unroll=4)

        if first:
            st_copy(1).start()
        else:
            st_copy(i - 1).wait()

            def repack(c, carry):
                repack_chunk(i - 1, c, range(H // 2))
                return carry

            jax.lax.fori_loop(0, D // 128, repack, 0)

            @pl.when(i == 1)
            def _():
                st_copy(2).start()

    branch_a(0, True)

    def phase1(i, carry):
        branch_a(i, False)
        return carry

    jax.lax.fori_loop(1, NCT, phase1, 0)
    misc[1].wait()
    for j in range(D // 128):
        wo_copy(j).wait()

    row = jax.lax.broadcasted_iota(jnp.int32, (ROWS, ROWS), 0)
    col = jax.lax.broadcasted_iota(jnp.int32, (ROWS, ROWS), 1)
    mask0 = ((col < M) | (col >= 16)) & ((row < 16) | (col <= row))
    mask1 = ((col < 16) | (col >= 24)) & ((row < M) | (col <= row))
    scale = DH ** -0.5

    def getw(m, g):
        return pltpu.bitcast(wqkv_s[m, g], bf16)

    def getwo(g):
        return jnp.concatenate([wo_s[j, g * GW:(g + 1) * GW, :] for j in range(D // 128)], axis=1)

    def attn(q, k, v, mask):
        outs = []
        for e in range(GH):
            sl = slice(e * 128, (e + 1) * 128)
            s = jax.lax.dot_general(q[:, sl], k[:, sl], (((1,), (1,)), ((), ())),
                                    preferred_element_type=f32)
            s = jnp.where(mask, s * scale, -1e9)
            mx = jnp.max(s, axis=-1, keepdims=True)
            ex = jnp.exp(s - mx)
            sm = jnp.sum(ex, axis=-1, keepdims=True)
            p = (ex / sm).astype(bf16)
            outs.append(jnp.dot(p, v[:, sl], preferred_element_type=f32))
        return jnp.concatenate(outs, axis=1)

    def out_copy(j):
        r0 = pl.multiple_of(j * 2 * SEG, 2 * SEG)
        return pltpu.make_async_copy(o_s.at[pl.ds(r0, 2 * SEG), :],
                                     out_hbm.at[pl.ds(r0, 2 * SEG), :], sem_out)

    def half_step(hb, even):
        ts, os_ = {}, {}
        acc = None
        for g in range(NG + LAG):
            cs = slice(g * GW, (g + 1) * GW)
            if g < NG:
                ts[g] = tuple(jnp.dot(hb, getw(m, g), preferred_element_type=f32) for m in range(3))
            if 1 <= g <= NG:
                a = g - 1
                ca = slice(a * GW, (a + 1) * GW)
                if even:
                    for m in range(3):
                        stash_s[m, :, ca] = ts[a][m][8:16]
                    q, k, v = (t.astype(bf16) for t in ts[a])
                    o = attn(q, k, v, mask0)
                    stash_s[3, :, ca] = o[40:48]
                    os_[a] = jnp.concatenate([o[0:8], o[16:40]], axis=0).astype(bf16)
                else:
                    q, k, v = (jnp.concatenate(
                        [jnp.concatenate([ts[a][m][0:8], stash_s[m, :, ca]], axis=0).astype(bf16),
                         ts[a][m].astype(bf16)], axis=0) for m in range(3))
                    o = attn(q, k, v, mask1)
                    os_[a] = jnp.concatenate([o[0:16], stash_s[3, :, ca], o[24:48]], axis=0).astype(bf16)
            if g >= LAG:
                d = jnp.dot(os_[g - LAG], getwo(g - LAG), preferred_element_type=f32)
                acc = d if acc is None else acc + d
        return acc

    def step(j, mem):
        @pl.when(j == XH // (2 * SEG) - 1)
        def _():
            misc[2].wait()

        r0 = pl.multiple_of(j * 2 * SEG, 2 * SEG)
        xa = x_s[pl.ds(r0, SEG), :]
        xb = x_s[pl.ds(r0 + SEG, 16), :].astype(f32)
        xc = x_s[pl.ds(r0 + SEG + 16, 16), :]
        hb = jnp.concatenate([jnp.concatenate([mem, xb[0:8]], axis=0).astype(bf16), xa], axis=0)
        acc0 = half_step(hb, True)
        hb = jnp.concatenate([jnp.concatenate([acc0[0:8], xb[8:16]], axis=0).astype(bf16), xc], axis=0)
        acc1 = half_step(hb, False)
        b = jnp.concatenate([acc0[8:32], acc1[16:24], acc1[8:16], acc1[24:48]], axis=0)
        xf = x_s[pl.ds(r0, 2 * SEG), :].astype(f32)
        gate = jnp.sum(xf * par_s[5:6, :], axis=-1, keepdims=True)
        gate = 1.0 / (1.0 + jnp.exp(-gate))
        res = gate * (xf * o_s[pl.ds(r0, 2 * SEG), :].astype(f32)) + (1.0 - gate) * b
        o_s[pl.ds(r0, 2 * SEG), :] = res.astype(bf16)
        out_copy(j).start()
        return acc1[0:8]

    jax.lax.fori_loop(0, NSEG // 2, step, mem0_ref[...].astype(f32))
    pltpu.make_async_copy(o_s, out_hbm, sem_out).wait()


@functools.partial(jax.jit, static_argnames=("B_seg_len",))
def pallas_gated_mix__ssm_conv_h3__memory_aug_recurrent_mem_tr__prompt_kernel(
    A_q, A_k, A_v, A_shift_k, A_ssm_k, A_ssm_D, B_x, B_mem0,
    B_Wq, B_Wk, B_Wv, B_Wo, B_seg_len, gate_w,
):
    assert B_seg_len == SEG
    bf16 = jnp.bfloat16
    f32 = jnp.float32
    hbm = pl.BlockSpec(memory_space=pl.ANY)
    vmem = pl.BlockSpec(memory_space=pltpu.VMEM)
    out = pl.pallas_call(
        _kernel,
        out_shape=jax.ShapeDtypeStruct((S, D), bf16),
        in_specs=[vmem] * 8 + [hbm] * 9,
        out_specs=hbm,
        scratch_shapes=[
            pltpu.VMEM((S, D), bf16),
            pltpu.VMEM((S, D), bf16),
            pltpu.VMEM((3, NG, D // 2, GW), jnp.uint32),
            pltpu.VMEM((D // 128, H * DH, 128), bf16),
            pltpu.VMEM((3, D // 128, 64 * H, DH), jnp.uint32),
            pltpu.VMEM((NCT, S, CT), bf16),
            pltpu.VMEM((NCT, S, CT), bf16),
            pltpu.VMEM((NCT, CT, S), bf16),
            pltpu.VMEM((CT // 128, 8 + S, 128), f32),
            pltpu.VMEM((CT // 128, S, 128), f32),
            pltpu.VMEM((48, 128, CT), bf16),
            pltpu.VMEM((48, CT, 128), bf16),
            pltpu.VMEM((48, 128, CT), bf16),
            pltpu.VMEM((32, 128, CT), f32),
            pltpu.VMEM((144, 128, 128), bf16),
            pltpu.VMEM((4, 8, H * DH), f32),
            pltpu.VMEM((8, D), f32),
            pltpu.SemaphoreType.DMA((3, NCT)),
            pltpu.SemaphoreType.DMA((3,)),
            pltpu.SemaphoreType.DMA((3,)),
            pltpu.SemaphoreType.DMA((D // 128,)),
            pltpu.SemaphoreType.DMA(()),
        ],
        compiler_params=pltpu.CompilerParams(vmem_limit_bytes=112 * 1024 * 1024),
    )(
        A_shift_k.T, A_ssm_D, gate_w, B_mem0.reshape(M, D), jnp.asarray(_GF8, bf16), jnp.asarray(_GI8, bf16),
        jnp.asarray(_CW), jnp.asarray(_CTW),
        A_q.reshape(S, D), A_k.reshape(S, D), A_v.reshape(S, D), A_ssm_k,
        B_Wq.reshape(D // 128, 128 * H, DH), B_Wk.reshape(D // 128, 128 * H, DH), B_Wv.reshape(D // 128, 128 * H, DH),
        B_Wo.reshape(H * DH, D), jnp.asarray(_FINV, bf16),
    )
    return out.reshape(1, S, D)
```

```python
import functools

import jax
import jax.numpy as jnp
import numpy as np
from jax.experimental import pallas as pl
from jax.experimental.pallas import tpu as pltpu

S, D = 2048, 1024
H, DH = 32, 128
M, SEG = 8, 32
NSEG = S // SEG
KS = 4
CT = 256
NCT = D // CT
GH = 4
NG = H // GH
GW = GH * DH
ROWS = 48
NFFT = 2 * S
XH = 256
ORDER = "swxqkpv"
LAG = 3


def _fft_constants():
    n1 = np.arange(16)
    k1 = np.arange(16)
    c = np.exp(-1j * np.pi * np.outer(2 * k1 + 1, n1) / 32.0)
    gf = np.concatenate([c.real, c.imag], axis=0)
    gi = np.concatenate([c.real.T, c.imag.T], axis=1) * (2.0 / NFFT)
    eye = np.eye(8)
    gf8 = np.kron(gf, eye)
    gi8 = np.kron(gi, eye)
    n2 = np.arange(128)
    w = np.exp(-2j * np.pi * np.outer(n2, n2) / 128.0)
    tw = np.exp(-2j * np.pi * np.outer(np.arange(16) + 0.5, n2) / NFFT)
    perm = 32 * (n2 // 32) + 4 * (n2 % 8) + (n2 // 8) % 4
    cw = np.stack([w.real[:, perm], w.imag[:, perm], w.real, w.imag])
    ctw = np.stack([tw.real[:, perm], tw.imag[:, perm], tw.real, tw.imag])
    inv = []
    for a in range(16):
        m = np.conj(w * tw[a][None, :]).T
        inv += [m.real, m.imag, m.real + m.imag]
    return tuple(np.asarray(t, np.float32) for t in (gf8, gi8, cw, ctw, np.stack(inv)))


_GF8, _GI8, _CW, _CTW, _FINV = _fft_constants()


def _kernel(taps_ref, d_ref, gw_ref, mem0_ref, gf_ref, gi_ref, cw_ref, ctw_ref,
            q_hbm, k_hbm, v_hbm, h_hbm, wq_hbm, wk_hbm, wv_hbm, wo_hbm, f_hbm,
            out_hbm,
            x_s, o_s, wqkv_s, wo_s, st_s, kin_s, vin_s, hin_s,
            kpad_s, vf_s, a_s, ah_s, y_s, b_s, f_s, stash_s, par_s,
            sem_in, sem_st, sem_misc, sem_wo, sem_out):
    bf16, f32 = jnp.bfloat16, jnp.float32

    def k_copy(i):
        c0 = pl.multiple_of(i * CT, CT)
        return pltpu.make_async_copy(k_hbm.at[:, pl.ds(c0, CT)], kin_s.at[i], sem_in.at[0, i])

    def v_copy(i):
        c0 = pl.multiple_of(i * CT, CT)
        return pltpu.make_async_copy(v_hbm.at[:, pl.ds(c0, CT)], vin_s.at[i], sem_in.at[1, i])

    def h_copy(i):
        c0 = pl.multiple_of(i * CT, CT)
        return pltpu.make_async_copy(h_hbm.at[pl.ds(c0, CT), :], hin_s.at[i], sem_in.at[2, i])

    def start_tile(i):
        k_copy(i).start()
        v_copy(i).start()
        h_copy(i).start()

    misc = (
        pltpu.make_async_copy(f_hbm, f_s.at[96:144], sem_misc.at[0]),
        pltpu.make_async_copy(q_hbm.at[0:XH], x_s.at[0:XH], sem_misc.at[1]),
        pltpu.make_async_copy(q_hbm.at[XH:S], x_s.at[XH:S], sem_misc.at[2]),
    )
    w_srcs = (wq_hbm, wk_hbm, wv_hbm)

    def st_copy(m):
        src = w_srcs[m] if isinstance(m, int) else w_srcs[0]
        return pltpu.make_async_copy(src, st_s.at[m].bitcast(bf16), sem_st.at[m])

    def wo_copy(j):
        return pltpu.make_async_copy(wo_hbm.at[:, pl.ds(j * 128, 128)], wo_s.at[j], sem_wo.at[j])

    k_copy(0).start()
    v_copy(0).start()

    def build_f(a, carry):
        for v in range(2):
            wr, wi = cw_ref[2 * v], cw_ref[2 * v + 1]
            tr, ti = ctw_ref[2 * v, pl.ds(a, 1), :], ctw_ref[2 * v + 1, pl.ds(a, 1), :]
            mr = wr * tr - wi * ti
            mi = wr * ti + wi * tr
            f_s[v * 48 + 3 * a] = mr.astype(bf16)
            f_s[v * 48 + 3 * a + 1] = mi.astype(bf16)
            f_s[v * 48 + 3 * a + 2] = (mr + mi).astype(bf16)
        return carry

    jax.lax.fori_loop(0, 16, build_f, 0)
    par_s[...] = jnp.concatenate(
        [taps_ref[...].astype(f32), d_ref[...].astype(f32).reshape(1, D), gw_ref[...].astype(f32).reshape(1, D),
         jnp.zeros((2, D), f32)], axis=0)
    gf = gf_ref[...]
    gi = gi_ref[...]
    kpad_s[:, 0:8, :] = jnp.zeros((CT // 128, 8, 128), f32)

    def repack_chunk(m, c, hps):
        r0 = pl.multiple_of(c * 64, 64)
        for hp in hps:
            w = st_s[m, c, pl.ds(hp, 128, stride=16), :]
            lo = pltpu.bitcast(w << 16, f32).astype(bf16)
            hi = pltpu.bitcast(w & jnp.uint32(0xFFFF0000), f32).astype(bf16)
            for hh, val in ((2 * hp, lo), (2 * hp + 1, hi)):
                g, e = hh // GH, hh % GH
                wqkv_s[m, g, pl.ds(r0, 64), e * 128:(e + 1) * 128] = pltpu.bitcast(val, jnp.uint32)

    def branch_a(i, first):
        slot = i
        c0 = pl.multiple_of(i * CT, CT)
        k_copy(i).wait()
        v_copy(i).wait()
        if first:
            h_copy(0).start()
            misc[0].start()
            start_tile(1)

        def cvt_body(r, carry):
            r0 = pl.multiple_of(r * 256, 256)
            kf = kin_s[slot, pl.ds(r0, 256), :].astype(f32)
            vf = vin_s[slot, pl.ds(r0, 256), :].astype(f32)
            for c in range(CT // 128):
                kpad_s[c, pl.ds(8 + r0, 256), :] = kf[:, c * 128:(c + 1) * 128]
                vf_s[c, pl.ds(r0, 256), :] = vf[:, c * 128:(c + 1) * 128]
            return carry

        jax.lax.fori_loop(0, S // 256, cvt_body, 0)


        pt = par_s[:, pl.ds(c0, CT)]
        taps = [pt[j:j + 1, :] for j in range(KS)]
        dvec = pt[4:5, :]

        def sload(ref, t0):
            return jnp.concatenate(
                [ref[c, pl.ds(t0, 8, stride=4), :] for c in range(CT // 128)], axis=1)

        for jj in range(8):
            outs = []
            for j in (2 * jj, 2 * jj + 1):
                blocks = []
                for n1 in range(16):
                    t0 = n1 * 128 + 32 * (j // 4) + j % 4
                    acc = sload(kpad_s, 8 + t0) * taps[0]
                    for t in range(1, KS):
                        acc = acc + sload(kpad_s, 8 + t0 - t) * taps[t]
                    blocks.append(acc * sload(vf_s, t0))
                rhs = jnp.concatenate(blocks, axis=0).astype(bf16)
                outs.append(jnp.dot(gf, rhs, preferred_element_type=f32))
            for ks in range(16):
                re, im = (jnp.concatenate([o[u * 8:(u + 1) * 8] for o in outs], axis=0)
                          for u in (ks, 16 + ks))
                for u, val in enumerate((re, im, re + im)):
                    a_s[3 * ks + u, jj * 16:(jj + 1) * 16, :] = val.astype(bf16)

        if first:
            st_copy(0).start()
        else:
            @pl.when(i == 1)
            def _():
                start_tile(3)

            @pl.when(i == 2)
            def _():
                misc[1].start()
                for j in range(D // 128):
                    wo_copy(j).start()
                misc[2].start()

        h_copy(i).wait()


        def h1_body(j, carry):
            j8 = pl.multiple_of(j * 16, 16)
            hv = hin_s[slot, pl.ds(j8, 16), :].astype(f32)
            lo, hi = hv[0:8], hv[8:16]
            blocks = [jnp.concatenate([lo[:, n1 * 128:(n1 + 1) * 128],
                                       hi[:, n1 * 128:(n1 + 1) * 128]], axis=1)
                      for n1 in range(16)]
            rhs = jnp.concatenate(blocks, axis=0).astype(bf16)
            out = jnp.dot(gf, rhs, preferred_element_type=f32)
            for ks in range(16):
                re, im = (jnp.concatenate(
                    [out[u * 8:(u + 1) * 8, 0:128], out[u * 8:(u + 1) * 8, 128:256]], axis=0)
                    for u in (ks, 16 + ks))
                for u, val in enumerate((re, im, re + im)):
                    ah_s[3 * ks + u, pl.ds(j8, 16), :] = val.astype(bf16)
            return carry

        jax.lax.fori_loop(0, CT // 16, h1_body, 0, unroll=8)

        def cmul3(lhs, rhs, nt):
            dims = (((1,), (1,)), ((), ())) if nt else (((1,), (0,)), ((), ()))
            t1, t2, t3 = (jax.lax.dot_general(lhs(u), rhs(u), dims, preferred_element_type=f32)
                          for u in range(3))
            return t1 - t2, t3 - t1 - t2

        def s2_body(k1, carry):
            xr, xi = cmul3(lambda u: f_s[3 * k1 + u], lambda u: a_s[3 * k1 + u], False)
            hr, hi = cmul3(lambda u: f_s[48 + 3 * k1 + u], lambda u: ah_s[3 * k1 + u], True)
            hr = hr + dvec
            yr = xr * hr - xi * hi
            yi = xr * hi + xi * hr
            for u, val in enumerate((yr, yi, yr + yi)):
                y_s[3 * k1 + u] = val.astype(bf16)
            return carry

        jax.lax.fori_loop(0, 16, s2_body, 0, unroll=8)

        if first:
            start_tile(2)
            misc[0].wait()

        def s3_body(k1, carry):
            br, bi = cmul3(lambda u: f_s[96 + 3 * k1 + u], lambda u: y_s[3 * k1 + u], False)
            b_s[k1] = br
            b_s[16 + k1] = bi
            return carry

        jax.lax.fori_loop(0, 16, s3_body, 0, unroll=8)

        def inv_body(jj, carry):
            j16 = pl.multiple_of(jj * 16, 16)
            ys = []
            for u in range(2):
                rhs = jnp.concatenate(
                    [b_s[ks, pl.ds(j16 + 8 * u, 8), :] for ks in range(32)], axis=0).astype(bf16)
                ys.append(jnp.dot(gi, rhs, preferred_element_type=f32))
            for n1 in range(16):
                r0 = pl.multiple_of(n1 * 128 + j16, 16)
                y = jnp.concatenate([ys[0][n1 * 8:(n1 + 1) * 8], ys[1][n1 * 8:(n1 + 1) * 8]], axis=0)
                o_s[pl.ds(r0, 16), pl.ds(c0, CT)] = y.astype(bf16)
            return carry

        jax.lax.fori_loop(0, 8, inv_body, 0, unroll=4)

        if first:
            st_copy(1).start()
        else:
            st_copy(i - 1).wait()

            def repack(c, carry):
                repack_chunk(i - 1, c, range(H // 2))
                return carry

            jax.lax.fori_loop(0, D // 128, repack, 0)

            @pl.when(i == 1)
            def _():
                st_copy(2).start()

    branch_a(0, True)

    def phase1(i, carry):
        branch_a(i, False)
        return carry

    jax.lax.fori_loop(1, NCT, phase1, 0)
    misc[1].wait()
    for j in range(D // 128):
        wo_copy(j).wait()

    row = jax.lax.broadcasted_iota(jnp.int32, (ROWS, ROWS), 0)
    col = jax.lax.broadcasted_iota(jnp.int32, (ROWS, ROWS), 1)
    mask0 = ((col < M) | (col >= 16)) & ((row < 16) | (col <= row))
    mask1 = ((col < 16) | (col >= 24)) & ((row < M) | (col <= row))
    scale = DH ** -0.5

    def getw(m, g):
        return pltpu.bitcast(wqkv_s[m, g], bf16)

    def getwo(g):
        return jnp.concatenate([wo_s[j, g * GW:(g + 1) * GW, :] for j in range(D // 128)], axis=1)

    def head_slices():
        return [slice(e * DH, (e + 1) * DH) for e in range(GH)]

    def scores(q, k):
        return [jax.lax.dot_general(q[:, sl], k[:, sl], (((1,), (1,)), ((), ())),
                                    preferred_element_type=f32) for sl in head_slices()]

    def softmax(s, mask):
        s = jnp.where(mask, s * scale, -1e9)
        ex = jnp.exp(s - jnp.max(s, axis=-1, keepdims=True))
        return (ex / jnp.sum(ex, axis=-1, keepdims=True)).astype(bf16)

    def out_copy(j):
        r0 = pl.multiple_of(j * 2 * SEG, 2 * SEG)
        return pltpu.make_async_copy(o_s.at[pl.ds(r0, 2 * SEG), :],
                                     out_hbm.at[pl.ds(r0, 2 * SEG), :], sem_out)

    def half_step(hb, even):
        mask = mask0 if even else mask1
        proj, full, sc, pr, os_ = {}, {}, {}, {}, {}
        acc = [None]

        def project(g, m):
            t = jnp.dot(hb, getw(m, g), preferred_element_type=f32)
            cs = slice(g * GW, (g + 1) * GW)
            if even:
                stash_s[m, :, cs] = t[8:16]
                full[g, m] = t.astype(bf16)
            else:
                top = jnp.concatenate([t[0:8], stash_s[m, :, cs]], axis=0).astype(bf16)
                full[g, m] = jnp.concatenate([top, t.astype(bf16)], axis=0)

        def do_scores(g):
            sc[g] = scores(full[g, 0], full[g, 1])

        def do_softmax(g):
            pr[g] = [softmax(s, mask) for s in sc[g]]

        def do_pv(g):
            o = jnp.concatenate(
                [jnp.dot(p, full[g, 2][:, sl], preferred_element_type=f32)
                 for p, sl in zip(pr[g], head_slices())], axis=1)
            cs = slice(g * GW, (g + 1) * GW)
            if even:
                stash_s[3, :, cs] = o[40:48]
                os_[g] = jnp.concatenate([o[0:8], o[16:40]], axis=0).astype(bf16)
            else:
                os_[g] = jnp.concatenate([o[0:16], stash_s[3, :, cs], o[24:48]], axis=0).astype(bf16)

        def do_out(g):
            d = jnp.dot(os_[g], getwo(g), preferred_element_type=f32)
            acc[0] = d if acc[0] is None else acc[0] + d

        stages = {
            "q": (0, functools.partial(project, m=0)), "k": (0, functools.partial(project, m=1)),
            "v": (0, functools.partial(project, m=2)), "s": (1, do_scores),
            "x": (1, do_softmax), "p": (1, do_pv), "w": (LAG, do_out),
        }
        for it in range(NG + LAG):
            for name in ORDER:
                lag, fn = stages[name]
                if 0 <= it - lag < NG:
                    fn(it - lag)
        return acc[0]

    def step(j, mem):
        @pl.when(j == XH // (2 * SEG) - 1)
        def _():
            misc[2].wait()

        r0 = pl.multiple_of(j * 2 * SEG, 2 * SEG)
        xa = x_s[pl.ds(r0, SEG), :]
        xb = x_s[pl.ds(r0 + SEG, 16), :].astype(f32)
        xc = x_s[pl.ds(r0 + SEG + 16, 16), :]
        hb = jnp.concatenate([jnp.concatenate([mem, xb[0:8]], axis=0).astype(bf16), xa], axis=0)
        acc0 = half_step(hb, True)
        hb = jnp.concatenate([jnp.concatenate([acc0[0:8], xb[8:16]], axis=0).astype(bf16), xc], axis=0)
        acc1 = half_step(hb, False)
        b = jnp.concatenate([acc0[8:32], acc1[16:24], acc1[8:16], acc1[24:48]], axis=0)
        xf = x_s[pl.ds(r0, 2 * SEG), :].astype(f32)
        gate = jnp.sum(xf * par_s[5:6, :], axis=-1, keepdims=True)
        gate = 1.0 / (1.0 + jnp.exp(-gate))
        res = gate * (xf * o_s[pl.ds(r0, 2 * SEG), :].astype(f32)) + (1.0 - gate) * b
        o_s[pl.ds(r0, 2 * SEG), :] = res.astype(bf16)
        out_copy(j).start()
        return acc1[0:8]

    jax.lax.fori_loop(0, NSEG // 2, step, mem0_ref[...].astype(f32))
    pltpu.make_async_copy(o_s, out_hbm, sem_out).wait()


@functools.partial(jax.jit, static_argnames=("B_seg_len",))
def pallas_gated_mix__ssm_conv_h3__memory_aug_recurrent_mem_tr__prompt_kernel(
    A_q, A_k, A_v, A_shift_k, A_ssm_k, A_ssm_D, B_x, B_mem0,
    B_Wq, B_Wk, B_Wv, B_Wo, B_seg_len, gate_w,
):
    assert B_seg_len == SEG
    bf16 = jnp.bfloat16
    f32 = jnp.float32
    hbm = pl.BlockSpec(memory_space=pl.ANY)
    vmem = pl.BlockSpec(memory_space=pltpu.VMEM)
    out = pl.pallas_call(
        _kernel,
        out_shape=jax.ShapeDtypeStruct((S, D), bf16),
        in_specs=[vmem] * 8 + [hbm] * 9,
        out_specs=hbm,
        scratch_shapes=[
            pltpu.VMEM((S, D), bf16),
            pltpu.VMEM((S, D), bf16),
            pltpu.VMEM((3, NG, D // 2, GW), jnp.uint32),
            pltpu.VMEM((D // 128, H * DH, 128), bf16),
            pltpu.VMEM((3, D // 128, 64 * H, DH), jnp.uint32),
            pltpu.VMEM((NCT, S, CT), bf16),
            pltpu.VMEM((NCT, S, CT), bf16),
            pltpu.VMEM((NCT, CT, S), bf16),
            pltpu.VMEM((CT // 128, 8 + S, 128), f32),
            pltpu.VMEM((CT // 128, S, 128), f32),
            pltpu.VMEM((48, 128, CT), bf16),
            pltpu.VMEM((48, CT, 128), bf16),
            pltpu.VMEM((48, 128, CT), bf16),
            pltpu.VMEM((32, 128, CT), f32),
            pltpu.VMEM((144, 128, 128), bf16),
            pltpu.VMEM((4, 8, H * DH), f32),
            pltpu.VMEM((8, D), f32),
            pltpu.SemaphoreType.DMA((3, NCT)),
            pltpu.SemaphoreType.DMA((3,)),
            pltpu.SemaphoreType.DMA((3,)),
            pltpu.SemaphoreType.DMA((D // 128,)),
            pltpu.SemaphoreType.DMA(()),
        ],
        compiler_params=pltpu.CompilerParams(vmem_limit_bytes=112 * 1024 * 1024),
    )(
        A_shift_k.T, A_ssm_D, gate_w, B_mem0.reshape(M, D), jnp.asarray(_GF8, bf16), jnp.asarray(_GI8, bf16),
        jnp.asarray(_CW), jnp.asarray(_CTW),
        A_q.reshape(S, D), A_k.reshape(S, D), A_v.reshape(S, D), A_ssm_k,
        B_Wq.reshape(D // 128, 128 * H, DH), B_Wk.reshape(D // 128, 128 * H, DH), B_Wv.reshape(D // 128, 128 * H, DH),
        B_Wo.reshape(H * DH, D), jnp.asarray(_FINV, bf16),
    )
    return out.reshape(1, S, D)
```

```python
import functools

import jax
import jax.numpy as jnp
import numpy as np
from jax.experimental import pallas as pl
from jax.experimental.pallas import tpu as pltpu

S, D = 2048, 1024
H, DH = 32, 128
M, SEG = 8, 32
NSEG = S // SEG
KS = 4
CT = 256
NCT = D // CT
GH = 4
NG = H // GH
GW = GH * DH
ROWS = 48
NFFT = 2 * S
XH = 256
XLAG = 1
PLAG = 2
LAG = 4
ORDER = "sqxkwvp"


def _fft_constants():
    n1 = np.arange(16)
    k1 = np.arange(16)
    c = np.exp(-1j * np.pi * np.outer(2 * k1 + 1, n1) / 32.0)
    gf = np.concatenate([c.real, c.imag], axis=0)
    gi = np.concatenate([c.real.T, c.imag.T], axis=1) * (2.0 / NFFT)
    eye = np.eye(8)
    gf8 = np.kron(gf, eye)
    gi8 = np.kron(gi, eye)
    n2 = np.arange(128)
    w = np.exp(-2j * np.pi * np.outer(n2, n2) / 128.0)
    tw = np.exp(-2j * np.pi * np.outer(np.arange(16) + 0.5, n2) / NFFT)
    perm = 32 * (n2 // 32) + 4 * (n2 % 8) + (n2 // 8) % 4
    cw = np.stack([w.real[:, perm], w.imag[:, perm], w.real, w.imag])
    ctw = np.stack([tw.real[:, perm], tw.imag[:, perm], tw.real, tw.imag])
    inv = []
    for a in range(16):
        m = np.conj(w * tw[a][None, :]).T
        inv += [m.real, m.imag, m.real + m.imag]
    return tuple(np.asarray(t, np.float32) for t in (gf8, gi8, cw, ctw, np.stack(inv)))


_GF8, _GI8, _CW, _CTW, _FINV = _fft_constants()


def _kernel(taps_ref, d_ref, gw_ref, mem0_ref, gf_ref, gi_ref, cw_ref, ctw_ref,
            q_hbm, k_hbm, v_hbm, h_hbm, wq_hbm, wk_hbm, wv_hbm, wo_hbm, f_hbm,
            out_hbm,
            x_s, o_s, wqkv_s, wo_s, st_s, kin_s, vin_s, hin_s,
            kpad_s, vf_s, a_s, ah_s, y_s, b_s, f_s, stash_s, par_s,
            sem_in, sem_st, sem_misc, sem_wo, sem_out):
    bf16, f32 = jnp.bfloat16, jnp.float32

    def k_copy(i):
        c0 = pl.multiple_of(i * CT, CT)
        return pltpu.make_async_copy(k_hbm.at[:, pl.ds(c0, CT)], kin_s.at[i], sem_in.at[0, i])

    def v_copy(i):
        c0 = pl.multiple_of(i * CT, CT)
        return pltpu.make_async_copy(v_hbm.at[:, pl.ds(c0, CT)], vin_s.at[i], sem_in.at[1, i])

    def h_copy(i):
        c0 = pl.multiple_of(i * CT, CT)
        return pltpu.make_async_copy(h_hbm.at[pl.ds(c0, CT), :], hin_s.at[i], sem_in.at[2, i])

    def start_tile(i):
        k_copy(i).start()
        v_copy(i).start()
        h_copy(i).start()

    misc = (
        pltpu.make_async_copy(f_hbm, f_s.at[96:144], sem_misc.at[0]),
        pltpu.make_async_copy(q_hbm.at[0:XH], x_s.at[0:XH], sem_misc.at[1]),
        pltpu.make_async_copy(q_hbm.at[XH:S], x_s.at[XH:S], sem_misc.at[2]),
    )
    w_srcs = (wq_hbm, wk_hbm, wv_hbm)

    def st_copy(m):
        src = w_srcs[m] if isinstance(m, int) else w_srcs[0]
        return pltpu.make_async_copy(src, st_s.at[m].bitcast(bf16), sem_st.at[m])

    def wo_copy(j):
        return pltpu.make_async_copy(wo_hbm.at[:, pl.ds(j * 128, 128)], wo_s.at[j], sem_wo.at[j])

    k_copy(0).start()
    v_copy(0).start()

    def build_f(a, carry):
        for v in range(2):
            wr, wi = cw_ref[2 * v], cw_ref[2 * v + 1]
            tr, ti = ctw_ref[2 * v, pl.ds(a, 1), :], ctw_ref[2 * v + 1, pl.ds(a, 1), :]
            mr = wr * tr - wi * ti
            mi = wr * ti + wi * tr
            f_s[v * 48 + 3 * a] = mr.astype(bf16)
            f_s[v * 48 + 3 * a + 1] = mi.astype(bf16)
            f_s[v * 48 + 3 * a + 2] = (mr + mi).astype(bf16)
        return carry

    jax.lax.fori_loop(0, 16, build_f, 0)
    par_s[...] = jnp.concatenate(
        [taps_ref[...].astype(f32), d_ref[...].astype(f32).reshape(1, D), gw_ref[...].astype(f32).reshape(1, D),
         jnp.zeros((2, D), f32)], axis=0)
    gf = gf_ref[...]
    gi = gi_ref[...]
    kpad_s[:, 0:8, :] = jnp.zeros((CT // 128, 8, 128), f32)

    def repack_chunk(m, c, hps):
        r0 = pl.multiple_of(c * 64, 64)
        for hp in hps:
            w = st_s[m, c, pl.ds(hp, 128, stride=16), :]
            lo = pltpu.bitcast(w << 16, f32).astype(bf16)
            hi = pltpu.bitcast(w & jnp.uint32(0xFFFF0000), f32).astype(bf16)
            for hh, val in ((2 * hp, lo), (2 * hp + 1, hi)):
                g, e = hh // GH, hh % GH
                wqkv_s[m, g, pl.ds(r0, 64), e * 128:(e + 1) * 128] = pltpu.bitcast(val, jnp.uint32)

    def branch_a(i, first):
        slot = i
        c0 = pl.multiple_of(i * CT, CT)
        k_copy(i).wait()
        v_copy(i).wait()
        if first:
            h_copy(0).start()
            misc[0].start()
            start_tile(1)

        def cvt_body(r, carry):
            r0 = pl.multiple_of(r * 256, 256)
            kf = kin_s[slot, pl.ds(r0, 256), :].astype(f32)
            vf = vin_s[slot, pl.ds(r0, 256), :].astype(f32)
            for c in range(CT // 128):
                kpad_s[c, pl.ds(8 + r0, 256), :] = kf[:, c * 128:(c + 1) * 128]
                vf_s[c, pl.ds(r0, 256), :] = vf[:, c * 128:(c + 1) * 128]
            return carry

        jax.lax.fori_loop(0, S // 256, cvt_body, 0)

        pt = par_s[:, pl.ds(c0, CT)]
        taps = [pt[j:j + 1, :] for j in range(KS)]
        dvec = pt[4:5, :]

        def sload(ref, t0):
            return jnp.concatenate(
                [ref[c, pl.ds(t0, 8, stride=4), :] for c in range(CT // 128)], axis=1)

        for jj in range(8):
            outs = []
            for j in (2 * jj, 2 * jj + 1):
                blocks = []
                for n1 in range(16):
                    t0 = n1 * 128 + 32 * (j // 4) + j % 4
                    acc = sload(kpad_s, 8 + t0) * taps[0]
                    for t in range(1, KS):
                        acc = acc + sload(kpad_s, 8 + t0 - t) * taps[t]
                    blocks.append(acc * sload(vf_s, t0))
                rhs = jnp.concatenate(blocks, axis=0).astype(bf16)
                outs.append(jnp.dot(gf, rhs, preferred_element_type=f32))
            for ks in range(16):
                re, im = (jnp.concatenate([o[u * 8:(u + 1) * 8] for o in outs], axis=0)
                          for u in (ks, 16 + ks))
                for u, val in enumerate((re, im, re + im)):
                    a_s[3 * ks + u, jj * 16:(jj + 1) * 16, :] = val.astype(bf16)

        if first:
            st_copy(0).start()
        else:
            @pl.when(i == 1)
            def _():
                start_tile(3)

            @pl.when(i == 2)
            def _():
                misc[1].start()
                for j in range(D // 128):
                    wo_copy(j).start()
                misc[2].start()

        h_copy(i).wait()

        def h1_body(j, carry):
            j8 = pl.multiple_of(j * 16, 16)
            hv = hin_s[slot, pl.ds(j8, 16), :].astype(f32)
            lo, hi = hv[0:8], hv[8:16]
            blocks = [jnp.concatenate([lo[:, n1 * 128:(n1 + 1) * 128],
                                       hi[:, n1 * 128:(n1 + 1) * 128]], axis=1)
                      for n1 in range(16)]
            rhs = jnp.concatenate(blocks, axis=0).astype(bf16)
            out = jnp.dot(gf, rhs, preferred_element_type=f32)
            for ks in range(16):
                re, im = (jnp.concatenate(
                    [out[u * 8:(u + 1) * 8, 0:128], out[u * 8:(u + 1) * 8, 128:256]], axis=0)
                    for u in (ks, 16 + ks))
                for u, val in enumerate((re, im, re + im)):
                    ah_s[3 * ks + u, pl.ds(j8, 16), :] = val.astype(bf16)
            return carry

        jax.lax.fori_loop(0, CT // 16, h1_body, 0, unroll=8)

        def cmul3(lhs, rhs, nt):
            dims = (((1,), (1,)), ((), ())) if nt else (((1,), (0,)), ((), ()))
            t1, t2, t3 = (jax.lax.dot_general(lhs(u), rhs(u), dims, preferred_element_type=f32)
                          for u in range(3))
            return t1 - t2, t3 - t1 - t2

        def s2_body(k1, carry):
            xr, xi = cmul3(lambda u: f_s[3 * k1 + u], lambda u: a_s[3 * k1 + u], False)
            hr, hi = cmul3(lambda u: f_s[48 + 3 * k1 + u], lambda u: ah_s[3 * k1 + u], True)
            hr = hr + dvec
            yr = xr * hr - xi * hi
            yi = xr * hi + xi * hr
            for u, val in enumerate((yr, yi, yr + yi)):
                y_s[3 * k1 + u] = val.astype(bf16)
            return carry

        jax.lax.fori_loop(0, 16, s2_body, 0, unroll=8)

        if first:
            start_tile(2)
            misc[0].wait()

        def s3_body(k1, carry):
            br, bi = cmul3(lambda u: f_s[96 + 3 * k1 + u], lambda u: y_s[3 * k1 + u], False)
            b_s[k1] = br
            b_s[16 + k1] = bi
            return carry

        jax.lax.fori_loop(0, 16, s3_body, 0, unroll=8)

        def inv_body(jj, carry):
            j16 = pl.multiple_of(jj * 16, 16)
            ys = []
            for u in range(2):
                rhs = jnp.concatenate(
                    [b_s[ks, pl.ds(j16 + 8 * u, 8), :] for ks in range(32)], axis=0).astype(bf16)
                ys.append(jnp.dot(gi, rhs, preferred_element_type=f32))
            for n1 in range(16):
                r0 = pl.multiple_of(n1 * 128 + j16, 16)
                y = jnp.concatenate([ys[0][n1 * 8:(n1 + 1) * 8], ys[1][n1 * 8:(n1 + 1) * 8]], axis=0)
                o_s[pl.ds(r0, 16), pl.ds(c0, CT)] = y.astype(bf16)
            return carry

        jax.lax.fori_loop(0, 8, inv_body, 0, unroll=4)

        if first:
            st_copy(1).start()
        else:
            st_copy(i - 1).wait()

            def repack(c, carry):
                repack_chunk(i - 1, c, range(H // 2))
                return carry

            jax.lax.fori_loop(0, D // 128, repack, 0)

            @pl.when(i == 1)
            def _():
                st_copy(2).start()

    branch_a(0, True)

    def phase1(i, carry):
        branch_a(i, False)
        return carry

    jax.lax.fori_loop(1, NCT, phase1, 0)
    misc[1].wait()
    for j in range(D // 128):
        wo_copy(j).wait()

    row = jax.lax.broadcasted_iota(jnp.int32, (ROWS, ROWS), 0)
    col = jax.lax.broadcasted_iota(jnp.int32, (ROWS, ROWS), 1)
    mask0 = ((col < M) | (col >= 16)) & ((row < 16) | (col <= row))
    mask1 = ((col < 16) | (col >= 24)) & ((row < M) | (col <= row))
    scale = DH ** -0.5

    def getw(m, g):
        return pltpu.bitcast(wqkv_s[m, g], bf16)

    def getwo(g):
        return jnp.concatenate([wo_s[j, g * GW:(g + 1) * GW, :] for j in range(D // 128)], axis=1)

    def head_slices():
        return [slice(e * DH, (e + 1) * DH) for e in range(GH)]

    def scores(q, k):
        return [jax.lax.dot_general(q[:, sl], k[:, sl], (((1,), (1,)), ((), ())),
                                    preferred_element_type=f32) for sl in head_slices()]

    def softmax(s, mask):
        s = jnp.where(mask, s * scale, -1e9)
        ex = jnp.exp(s - jnp.max(s, axis=-1, keepdims=True))
        return (ex / jnp.sum(ex, axis=-1, keepdims=True)).astype(bf16)

    def out_copy(j):
        r0 = pl.multiple_of(j * 2 * SEG, 2 * SEG)
        return pltpu.make_async_copy(o_s.at[pl.ds(r0, 2 * SEG), :],
                                     out_hbm.at[pl.ds(r0, 2 * SEG), :], sem_out)

    def half_step(hb, even):
        mask = mask0 if even else mask1
        proj, full, sc, pr, os_ = {}, {}, {}, {}, {}
        acc = [None]

        def project(g, m):
            t = jnp.dot(hb, getw(m, g), preferred_element_type=f32)
            cs = slice(g * GW, (g + 1) * GW)
            if even:
                stash_s[m, :, cs] = t[8:16]
                full[g, m] = t.astype(bf16)
            else:
                top = jnp.concatenate([t[0:8], stash_s[m, :, cs]], axis=0).astype(bf16)
                full[g, m] = jnp.concatenate([top, t.astype(bf16)], axis=0)

        def do_scores(g):
            sc[g] = scores(full[g, 0], full[g, 1])

        def do_softmax(g):
            pr[g] = [softmax(s, mask) for s in sc[g]]

        def do_pv(g):
            o = jnp.concatenate(
                [jnp.dot(p, full[g, 2][:, sl], preferred_element_type=f32)
                 for p, sl in zip(pr[g], head_slices())], axis=1)
            cs = slice(g * GW, (g + 1) * GW)
            if even:
                stash_s[3, :, cs] = o[40:48]
                os_[g] = jnp.concatenate([o[0:8], o[16:40]], axis=0).astype(bf16)
            else:
                os_[g] = jnp.concatenate([o[0:16], stash_s[3, :, cs], o[24:48]], axis=0).astype(bf16)

        def do_out(g):
            d = jnp.dot(os_[g], getwo(g), preferred_element_type=f32)
            acc[0] = d if acc[0] is None else acc[0] + d

        stages = {
            "q": (0, functools.partial(project, m=0)), "k": (0, functools.partial(project, m=1)),
            "v": (0, functools.partial(project, m=2)), "s": (1, do_scores),
            "x": (XLAG, do_softmax), "p": (PLAG, do_pv), "w": (LAG, do_out),
        }
        for it in range(NG + LAG):
            for name in ORDER:
                lag, fn = stages[name]
                if 0 <= it - lag < NG:
                    fn(it - lag)
        return acc[0]

    def step(j, mem):
        @pl.when(j == XH // (2 * SEG) - 1)
        def _():
            misc[2].wait()

        r0 = pl.multiple_of(j * 2 * SEG, 2 * SEG)
        xa = x_s[pl.ds(r0, SEG), :]
        xb = x_s[pl.ds(r0 + SEG, 16), :].astype(f32)
        xc = x_s[pl.ds(r0 + SEG + 16, 16), :]
        hb = jnp.concatenate([jnp.concatenate([mem, xb[0:8]], axis=0).astype(bf16), xa], axis=0)
        acc0 = half_step(hb, True)
        hb = jnp.concatenate([jnp.concatenate([acc0[0:8], xb[8:16]], axis=0).astype(bf16), xc], axis=0)
        acc1 = half_step(hb, False)
        b = jnp.concatenate([acc0[8:32], acc1[16:24], acc1[8:16], acc1[24:48]], axis=0)
        xf = x_s[pl.ds(r0, 2 * SEG), :].astype(f32)
        gate = jnp.sum(xf * par_s[5:6, :], axis=-1, keepdims=True)
        gate = 1.0 / (1.0 + jnp.exp(-gate))
        res = gate * (xf * o_s[pl.ds(r0, 2 * SEG), :].astype(f32)) + (1.0 - gate) * b
        o_s[pl.ds(r0, 2 * SEG), :] = res.astype(bf16)
        out_copy(j).start()
        return acc1[0:8]

    jax.lax.fori_loop(0, NSEG // 2, step, mem0_ref[...].astype(f32))
    pltpu.make_async_copy(o_s, out_hbm, sem_out).wait()


@functools.partial(jax.jit, static_argnames=("B_seg_len",))
def pallas_gated_mix__ssm_conv_h3__memory_aug_recurrent_mem_tr__prompt_kernel(
    A_q, A_k, A_v, A_shift_k, A_ssm_k, A_ssm_D, B_x, B_mem0,
    B_Wq, B_Wk, B_Wv, B_Wo, B_seg_len, gate_w,
):
    assert B_seg_len == SEG
    bf16 = jnp.bfloat16
    f32 = jnp.float32
    hbm = pl.BlockSpec(memory_space=pl.ANY)
    vmem = pl.BlockSpec(memory_space=pltpu.VMEM)
    out = pl.pallas_call(
        _kernel,
        out_shape=jax.ShapeDtypeStruct((S, D), bf16),
        in_specs=[vmem] * 8 + [hbm] * 9,
        out_specs=hbm,
        scratch_shapes=[
            pltpu.VMEM((S, D), bf16),
            pltpu.VMEM((S, D), bf16),
            pltpu.VMEM((3, NG, D // 2, GW), jnp.uint32),
            pltpu.VMEM((D // 128, H * DH, 128), bf16),
            pltpu.VMEM((3, D // 128, 64 * H, DH), jnp.uint32),
            pltpu.VMEM((NCT, S, CT), bf16),
            pltpu.VMEM((NCT, S, CT), bf16),
            pltpu.VMEM((NCT, CT, S), bf16),
            pltpu.VMEM((CT // 128, 8 + S, 128), f32),
            pltpu.VMEM((CT // 128, S, 128), f32),
            pltpu.VMEM((48, 128, CT), bf16),
            pltpu.VMEM((48, CT, 128), bf16),
            pltpu.VMEM((48, 128, CT), bf16),
            pltpu.VMEM((32, 128, CT), f32),
            pltpu.VMEM((144, 128, 128), bf16),
            pltpu.VMEM((4, 8, H * DH), f32),
            pltpu.VMEM((8, D), f32),
            pltpu.SemaphoreType.DMA((3, NCT)),
            pltpu.SemaphoreType.DMA((3,)),
            pltpu.SemaphoreType.DMA((3,)),
            pltpu.SemaphoreType.DMA((D // 128,)),
            pltpu.SemaphoreType.DMA(()),
        ],
        compiler_params=pltpu.CompilerParams(vmem_limit_bytes=112 * 1024 * 1024),
    )(
        A_shift_k.T, A_ssm_D, gate_w, B_mem0.reshape(M, D), jnp.asarray(_GF8, bf16), jnp.asarray(_GI8, bf16),
        jnp.asarray(_CW), jnp.asarray(_CTW),
        A_q.reshape(S, D), A_k.reshape(S, D), A_v.reshape(S, D), A_ssm_k,
        B_Wq.reshape(D // 128, 128 * H, DH), B_Wk.reshape(D // 128, 128 * H, DH), B_Wv.reshape(D // 128, 128 * H, DH),
        B_Wo.reshape(H * DH, D), jnp.asarray(_FINV, bf16),
    )
    return out.reshape(1, S, D)
```

```python
import functools

import jax
import jax.numpy as jnp
import numpy as np
from jax.experimental import pallas as pl
from jax.experimental.pallas import tpu as pltpu

S, D = 2048, 1024
H, DH = 32, 128
M, SEG = 8, 32
NSEG = S // SEG
KS = 4
CT = 256
NCT = D // CT
GH = 4
NG = H // GH
GW = GH * DH
ROWS = 48
NFFT = 2 * S
XH = 256
XLAG = 1
PLAG = 2
LAG = 4
ORDER = "sqxkwvp"


def _fft_constants():
    n1 = np.arange(16)
    k1 = np.arange(16)
    c = np.exp(-1j * np.pi * np.outer(2 * k1 + 1, n1) / 32.0)
    gf = np.concatenate([c.real, c.imag], axis=0)
    gi = np.concatenate([c.real.T, c.imag.T], axis=1) * (2.0 / NFFT)
    eye = np.eye(8)
    gf8 = np.kron(gf, eye)
    gi8 = np.kron(gi, eye)
    n2 = np.arange(128)
    w = np.exp(-2j * np.pi * np.outer(n2, n2) / 128.0)
    tw = np.exp(-2j * np.pi * np.outer(np.arange(16) + 0.5, n2) / NFFT)
    perm = 32 * (n2 // 32) + 4 * (n2 % 8) + (n2 // 8) % 4
    cw = np.stack([w.real[:, perm], w.imag[:, perm], w.real, w.imag])
    ctw = np.stack([tw.real[:, perm], tw.imag[:, perm], tw.real, tw.imag])
    return tuple(np.asarray(t, np.float32) for t in (gf8, gi8, cw, ctw))


_GF8, _GI8, _CW, _CTW = _fft_constants()


def _kernel(taps_ref, d_ref, gw_ref, mem0_ref, gf_ref, gi_ref, cw_ref, ctw_ref,
            q_hbm, k_hbm, v_hbm, h_hbm, wq_hbm, wk_hbm, wv_hbm, wo_hbm,
            out_hbm,
            x_s, o_s, wqkv_s, wo_s, st_s, kin_s, vin_s, hin_s,
            kpad_s, vf_s, a_s, ah_s, y_s, b_s, f_s, stash_s, par_s,
            sem_in, sem_st, sem_misc, sem_wo, sem_out):
    bf16, f32 = jnp.bfloat16, jnp.float32

    def k_copy(i):
        c0 = pl.multiple_of(i * CT, CT)
        return pltpu.make_async_copy(k_hbm.at[:, pl.ds(c0, CT)], kin_s.at[i], sem_in.at[0, i])

    def v_copy(i):
        c0 = pl.multiple_of(i * CT, CT)
        return pltpu.make_async_copy(v_hbm.at[:, pl.ds(c0, CT)], vin_s.at[i], sem_in.at[1, i])

    def h_copy(i):
        c0 = pl.multiple_of(i * CT, CT)
        return pltpu.make_async_copy(h_hbm.at[pl.ds(c0, CT), :], hin_s.at[i], sem_in.at[2, i])

    def start_tile(i):
        k_copy(i).start()
        v_copy(i).start()
        h_copy(i).start()

    misc = (
        pltpu.make_async_copy(q_hbm.at[0:XH], x_s.at[0:XH], sem_misc.at[0]),
        pltpu.make_async_copy(q_hbm.at[XH:S], x_s.at[XH:S], sem_misc.at[1]),
    )
    w_srcs = (wq_hbm, wk_hbm, wv_hbm)

    def st_copy(m):
        src = w_srcs[m] if isinstance(m, int) else w_srcs[0]
        return pltpu.make_async_copy(src, st_s.at[m].bitcast(bf16), sem_st.at[m])

    def wo_copy(j):
        return pltpu.make_async_copy(wo_hbm.at[:, pl.ds(j * 128, 128)], wo_s.at[j], sem_wo.at[j])

    k_copy(0).start()
    v_copy(0).start()
    h_copy(0).start()

    def build_f(a, carry):
        for v in range(2):
            wr, wi = cw_ref[2 * v], cw_ref[2 * v + 1]
            tr, ti = ctw_ref[2 * v, pl.ds(a, 1), :], ctw_ref[2 * v + 1, pl.ds(a, 1), :]
            mr = wr * tr - wi * ti
            mi = wr * ti + wi * tr
            f_s[v * 48 + 3 * a] = mr.astype(bf16)
            f_s[v * 48 + 3 * a + 1] = mi.astype(bf16)
            f_s[v * 48 + 3 * a + 2] = (mr + mi).astype(bf16)
            if v == 1:
                pr, qi = mr.T, -(mi.T)
                f_s[96 + 3 * a] = pr.astype(bf16)
                f_s[96 + 3 * a + 1] = qi.astype(bf16)
                f_s[96 + 3 * a + 2] = (pr + qi).astype(bf16)
        return carry

    jax.lax.fori_loop(0, 16, build_f, 0)
    par_s[...] = jnp.concatenate(
        [taps_ref[...].astype(f32), d_ref[...].astype(f32).reshape(1, D), gw_ref[...].astype(f32).reshape(1, D),
         jnp.zeros((2, D), f32)], axis=0)
    gf = gf_ref[...]
    gi = gi_ref[...]
    kpad_s[:, 0:8, :] = jnp.zeros((CT // 128, 8, 128), f32)

    def repack_chunk(m, c):
        r0 = pl.multiple_of(c * 32, 32)
        for hp in range(H // 2):
            w = st_s[m, c, pl.ds(hp, 64, stride=16), :]
            lo = pltpu.bitcast(w << 16, f32).astype(bf16)
            hi = pltpu.bitcast(w & jnp.uint32(0xFFFF0000), f32).astype(bf16)
            for hh, val in ((2 * hp, lo), (2 * hp + 1, hi)):
                g, e = hh // GH, hh % GH
                wqkv_s[m, g, pl.ds(r0, 32), e * 128:(e + 1) * 128] = pltpu.bitcast(val, jnp.uint32)

    def branch_a(i, first):
        slot = i
        c0 = pl.multiple_of(i * CT, CT)
        k_copy(i).wait()
        v_copy(i).wait()
        if first:
            start_tile(1)
            st_copy(0).start()

        def cvt_body(r, carry):
            r0 = pl.multiple_of(r * 256, 256)
            kf = kin_s[slot, pl.ds(r0, 256), :].astype(f32)
            vf = vin_s[slot, pl.ds(r0, 256), :].astype(f32)
            for c in range(CT // 128):
                kpad_s[c, pl.ds(8 + r0, 256), :] = kf[:, c * 128:(c + 1) * 128]
                vf_s[c, pl.ds(r0, 256), :] = vf[:, c * 128:(c + 1) * 128]
            return carry

        jax.lax.fori_loop(0, S // 256, cvt_body, 0)

        pt = par_s[:, pl.ds(c0, CT)]
        taps = [pt[j:j + 1, :] for j in range(KS)]
        dvec = pt[4:5, :]

        def sload(ref, t0):
            return jnp.concatenate(
                [ref[c, pl.ds(t0, 8, stride=4), :] for c in range(CT // 128)], axis=1)

        for jj in range(8):
            outs = []
            for j in (2 * jj, 2 * jj + 1):
                blocks = []
                for n1 in range(16):
                    t0 = n1 * 128 + 32 * (j // 4) + j % 4
                    acc = sload(kpad_s, 8 + t0) * taps[0]
                    for t in range(1, KS):
                        acc = acc + sload(kpad_s, 8 + t0 - t) * taps[t]
                    blocks.append(acc * sload(vf_s, t0))
                rhs = jnp.concatenate(blocks, axis=0).astype(bf16)
                outs.append(jnp.dot(gf, rhs, preferred_element_type=f32))
            for ks in range(16):
                re, im = (jnp.concatenate([o[u * 8:(u + 1) * 8] for o in outs], axis=0)
                          for u in (ks, 16 + ks))
                for u, val in enumerate((re, im, re + im)):
                    a_s[3 * ks + u, jj * 16:(jj + 1) * 16, :] = val.astype(bf16)

        if not first:
            @pl.when(i == 1)
            def _():
                start_tile(3)

            @pl.when(i == 2)
            def _():
                misc[0].start()
                for j in range(D // 128):
                    wo_copy(j).start()

        h_copy(i).wait()

        def h1_body(j, carry):
            j8 = pl.multiple_of(j * 16, 16)
            hv = hin_s[slot, pl.ds(j8, 16), :].astype(f32)
            lo, hi = hv[0:8], hv[8:16]
            blocks = [jnp.concatenate([lo[:, n1 * 128:(n1 + 1) * 128],
                                       hi[:, n1 * 128:(n1 + 1) * 128]], axis=1)
                      for n1 in range(16)]
            rhs = jnp.concatenate(blocks, axis=0).astype(bf16)
            out = jnp.dot(gf, rhs, preferred_element_type=f32)
            for ks in range(16):
                re, im = (jnp.concatenate(
                    [out[u * 8:(u + 1) * 8, 0:128], out[u * 8:(u + 1) * 8, 128:256]], axis=0)
                    for u in (ks, 16 + ks))
                for u, val in enumerate((re, im, re + im)):
                    ah_s[3 * ks + u, pl.ds(j8, 16), :] = val.astype(bf16)
            return carry

        jax.lax.fori_loop(0, CT // 16, h1_body, 0, unroll=8)

        def cmul3(lhs, rhs, nt):
            dims = (((1,), (1,)), ((), ())) if nt else (((1,), (0,)), ((), ()))
            t1, t2, t3 = (jax.lax.dot_general(lhs(u), rhs(u), dims, preferred_element_type=f32)
                          for u in range(3))
            return t1 - t2, t3 - t1 - t2

        def s2_body(k1, carry):
            xr, xi = cmul3(lambda u: f_s[3 * k1 + u], lambda u: a_s[3 * k1 + u], False)
            hr, hi = cmul3(lambda u: f_s[48 + 3 * k1 + u], lambda u: ah_s[3 * k1 + u], True)
            if not first:
                repack_chunk(i - 1, k1)
            hr = hr + dvec
            yr = xr * hr - xi * hi
            yi = xr * hi + xi * hr
            for u, val in enumerate((yr, yi, yr + yi)):
                y_s[3 * k1 + u] = val.astype(bf16)
            return carry

        if not first:
            st_copy(i - 1).wait()
        jax.lax.fori_loop(0, 16, s2_body, 0, unroll=8)

        if first:
            start_tile(2)

        def s3_body(k1, carry):
            br, bi = cmul3(lambda u: f_s[96 + 3 * k1 + u], lambda u: y_s[3 * k1 + u], False)
            b_s[k1] = br
            b_s[16 + k1] = bi
            return carry

        jax.lax.fori_loop(0, 16, s3_body, 0, unroll=8)

        def inv_body(jj, carry):
            j16 = pl.multiple_of(jj * 16, 16)
            ys = []
            for u in range(2):
                rhs = jnp.concatenate(
                    [b_s[ks, pl.ds(j16 + 8 * u, 8), :] for ks in range(32)], axis=0).astype(bf16)
                ys.append(jnp.dot(gi, rhs, preferred_element_type=f32))
            for n1 in range(16):
                r0 = pl.multiple_of(n1 * 128 + j16, 16)
                y = jnp.concatenate([ys[0][n1 * 8:(n1 + 1) * 8], ys[1][n1 * 8:(n1 + 1) * 8]], axis=0)
                o_s[pl.ds(r0, 16), pl.ds(c0, CT)] = y.astype(bf16)
            return carry

        jax.lax.fori_loop(0, 8, inv_body, 0, unroll=4)

        if first:
            st_copy(1).start()
        else:
            @pl.when(i == 1)
            def _():
                st_copy(2).start()

    branch_a(0, True)

    def phase1(i, carry):
        branch_a(i, False)
        return carry

    jax.lax.fori_loop(1, NCT, phase1, 0)
    misc[0].wait()
    misc[1].start()
    for j in range(D // 128):
        wo_copy(j).wait()

    row = jax.lax.broadcasted_iota(jnp.int32, (ROWS, ROWS), 0)
    col = jax.lax.broadcasted_iota(jnp.int32, (ROWS, ROWS), 1)
    mask0 = ((col < M) | (col >= 16)) & ((row < 16) | (col <= row))
    mask1 = ((col < 16) | (col >= 24)) & ((row < M) | (col <= row))
    scale = DH ** -0.5

    def getw(m, g):
        return pltpu.bitcast(wqkv_s[m, g], bf16)

    def getwo(g):
        return jnp.concatenate([wo_s[j, g * GW:(g + 1) * GW, :] for j in range(D // 128)], axis=1)

    def head_slices():
        return [slice(e * DH, (e + 1) * DH) for e in range(GH)]

    def scores(q, k):
        return [jax.lax.dot_general(q[:, sl], k[:, sl], (((1,), (1,)), ((), ())),
                                    preferred_element_type=f32) for sl in head_slices()]

    def softmax(s, mask):
        s = jnp.where(mask, s * scale, -1e9)
        ex = jnp.exp(s - jnp.max(s, axis=-1, keepdims=True))
        return (ex / jnp.sum(ex, axis=-1, keepdims=True)).astype(bf16)

    def out_copy(j):
        r0 = pl.multiple_of(j * 2 * SEG, 2 * SEG)
        return pltpu.make_async_copy(o_s.at[pl.ds(r0, 2 * SEG), :],
                                     out_hbm.at[pl.ds(r0, 2 * SEG), :], sem_out)

    def half_step(hb, even):
        mask = mask0 if even else mask1
        proj, full, sc, pr, os_ = {}, {}, {}, {}, {}
        acc = [None]

        def project(g, m):
            t = jnp.dot(hb, getw(m, g), preferred_element_type=f32)
            cs = slice(g * GW, (g + 1) * GW)
            if even:
                stash_s[m, :, cs] = t[8:16]
                full[g, m] = t.astype(bf16)
            else:
                top = jnp.concatenate([t[0:8], stash_s[m, :, cs]], axis=0).astype(bf16)
                full[g, m] = jnp.concatenate([top, t.astype(bf16)], axis=0)

        def do_scores(g):
            sc[g] = scores(full[g, 0], full[g, 1])

        def do_softmax(g):
            pr[g] = [softmax(s, mask) for s in sc[g]]

        def do_pv(g):
            o = jnp.concatenate(
                [jnp.dot(p, full[g, 2][:, sl], preferred_element_type=f32)
                 for p, sl in zip(pr[g], head_slices())], axis=1)
            cs = slice(g * GW, (g + 1) * GW)
            if even:
                stash_s[3, :, cs] = o[40:48]
                os_[g] = jnp.concatenate([o[0:8], o[16:40]], axis=0).astype(bf16)
            else:
                os_[g] = jnp.concatenate([o[0:16], stash_s[3, :, cs], o[24:48]], axis=0).astype(bf16)

        def do_out(g):
            d = jnp.dot(os_[g], getwo(g), preferred_element_type=f32)
            acc[0] = d if acc[0] is None else acc[0] + d

        stages = {
            "q": (0, functools.partial(project, m=0)), "k": (0, functools.partial(project, m=1)),
            "v": (0, functools.partial(project, m=2)), "s": (1, do_scores),
            "x": (XLAG, do_softmax), "p": (PLAG, do_pv), "w": (LAG, do_out),
        }
        for it in range(NG + LAG):
            for name in ORDER:
                lag, fn = stages[name]
                if 0 <= it - lag < NG:
                    fn(it - lag)
        return acc[0]

    def step(j, mem):
        @pl.when(j == XH // (2 * SEG) - 1)
        def _():
            misc[1].wait()

        r0 = pl.multiple_of(j * 2 * SEG, 2 * SEG)
        xa = x_s[pl.ds(r0, SEG), :]
        xb = x_s[pl.ds(r0 + SEG, 16), :].astype(f32)
        xc = x_s[pl.ds(r0 + SEG + 16, 16), :]
        hb = jnp.concatenate([jnp.concatenate([mem, xb[0:8]], axis=0).astype(bf16), xa], axis=0)
        acc0 = half_step(hb, True)
        hb = jnp.concatenate([jnp.concatenate([acc0[0:8], xb[8:16]], axis=0).astype(bf16), xc], axis=0)
        acc1 = half_step(hb, False)
        b = jnp.concatenate([acc0[8:32], acc1[16:24], acc1[8:16], acc1[24:48]], axis=0)
        xf = x_s[pl.ds(r0, 2 * SEG), :].astype(f32)
        gate = jnp.sum(xf * par_s[5:6, :], axis=-1, keepdims=True)
        gate = 1.0 / (1.0 + jnp.exp(-gate))
        res = gate * (xf * o_s[pl.ds(r0, 2 * SEG), :].astype(f32)) + (1.0 - gate) * b
        o_s[pl.ds(r0, 2 * SEG), :] = res.astype(bf16)
        out_copy(j).start()
        return acc1[0:8]

    jax.lax.fori_loop(0, NSEG // 2, step, mem0_ref[...].astype(f32))
    pltpu.make_async_copy(o_s, out_hbm, sem_out).wait()


@functools.partial(jax.jit, static_argnames=("B_seg_len",))
def pallas_gated_mix__ssm_conv_h3__memory_aug_recurrent_mem_tr__prompt_kernel(
    A_q, A_k, A_v, A_shift_k, A_ssm_k, A_ssm_D, B_x, B_mem0,
    B_Wq, B_Wk, B_Wv, B_Wo, B_seg_len, gate_w,
):
    assert B_seg_len == SEG
    bf16 = jnp.bfloat16
    f32 = jnp.float32
    hbm = pl.BlockSpec(memory_space=pl.ANY)
    vmem = pl.BlockSpec(memory_space=pltpu.VMEM)
    out = pl.pallas_call(
        _kernel,
        out_shape=jax.ShapeDtypeStruct((S, D), bf16),
        in_specs=[vmem] * 8 + [hbm] * 8,
        out_specs=hbm,
        scratch_shapes=[
            pltpu.VMEM((S, D), bf16),
            pltpu.VMEM((S, D), bf16),
            pltpu.VMEM((3, NG, D // 2, GW), jnp.uint32),
            pltpu.VMEM((D // 128, H * DH, 128), bf16),
            pltpu.VMEM((3, D // 64, 32 * H, DH), jnp.uint32),
            pltpu.VMEM((NCT, S, CT), bf16),
            pltpu.VMEM((NCT, S, CT), bf16),
            pltpu.VMEM((NCT, CT, S), bf16),
            pltpu.VMEM((CT // 128, 8 + S, 128), f32),
            pltpu.VMEM((CT // 128, S, 128), f32),
            pltpu.VMEM((48, 128, CT), bf16),
            pltpu.VMEM((48, CT, 128), bf16),
            pltpu.VMEM((48, 128, CT), bf16),
            pltpu.VMEM((32, 128, CT), f32),
            pltpu.VMEM((144, 128, 128), bf16),
            pltpu.VMEM((4, 8, H * DH), f32),
            pltpu.VMEM((8, D), f32),
            pltpu.SemaphoreType.DMA((3, NCT)),
            pltpu.SemaphoreType.DMA((3,)),
            pltpu.SemaphoreType.DMA((2,)),
            pltpu.SemaphoreType.DMA((D // 128,)),
            pltpu.SemaphoreType.DMA(()),
        ],
        compiler_params=pltpu.CompilerParams(vmem_limit_bytes=112 * 1024 * 1024),
    )(
        A_shift_k.T, A_ssm_D, gate_w, B_mem0.reshape(M, D), jnp.asarray(_GF8, bf16), jnp.asarray(_GI8, bf16),
        jnp.asarray(_CW), jnp.asarray(_CTW),
        A_q.reshape(S, D), A_k.reshape(S, D), A_v.reshape(S, D), A_ssm_k,
        B_Wq.reshape(D // 64, 64 * H, DH), B_Wk.reshape(D // 64, 64 * H, DH), B_Wv.reshape(D // 64, 64 * H, DH),
        B_Wo.reshape(H * DH, D),
    )
    return out.reshape(1, S, D)
```
